```python
import jax
import jax.numpy as jnp

def _softmax(x, axis=-1):
    return jax.nn.softmax(x, axis=axis)

def _gelu(x):
    return jax.nn.gelu(x, approximate=True)

def _silu(x):
    return jax.nn.silu(x)

def _sigmoid(x):
    return jax.nn.sigmoid(x)

def _layernorm(x, axis=-1, eps=1e-05):
    m = jnp.mean(x, axis=axis, keepdims=True)
    v = jnp.var(x, axis=axis, keepdims=True)
    return (x - m) / jnp.sqrt(v + eps)

def _scatter_add(tgt, idx, src, axis=0):
    return tgt.at[idx].add(src)

def _segment_sum(src, seg, n):
    return jax.ops.segment_sum(src, seg, n)

class _Rng:

    def __init__(self, key):
        self._k = key

    def _next(self):
        self._k, sub = jax.random.split(self._k)
        return sub

    def normal(self, shape):
        return jax.random.normal(self._next(), shape, dtype=jnp.bfloat16)

    def randint(self, lo, hi, shape):
        return jax.random.randint(self._next(), shape, lo, hi, dtype=jnp.int32)

    def uniform(self, shape, lo=0.0, hi=1.0):
        return jax.random.uniform(self._next(), shape, jnp.bfloat16, lo, hi)

    def permutation(self, n):
        return jax.random.permutation(self._next(), n)
kernel_name = 'recurrent_scan__memory_aug_recurrent_mem_tr__moe_arch_mod__prompt'

def setup_inputs():
    _rng = _Rng(jax.random.key(int.from_bytes(__import__("os").urandom(4), "little")))
    _w = lambda a: (lambda t: t.astype(jnp.bfloat16) if jnp.issubdtype(t.dtype, jnp.floating) else t)(jnp.asarray(a))

    def _A_setup():
        B, S, Dm = (1, 2048, 640)
        H, Dh = (32, 128)
        M, seg = (8, 32)
        seg = min(seg, S)
        S = S // seg * seg
        return {'x': _w((lambda *s: _rng.normal(s) * 0.05)(B, S, Dm)), 'mem0': _w((lambda *s: _rng.normal(s) * 0.05)(B, M, Dm)), 'Wq': _w((lambda *s: _rng.normal(s) * 0.05)(Dm, H, Dh) * Dm ** (-0.5)), 'Wk': _w((lambda *s: _rng.normal(s) * 0.05)(Dm, H, Dh) * Dm ** (-0.5)), 'Wv': _w((lambda *s: _rng.normal(s) * 0.05)(Dm, H, Dh) * Dm ** (-0.5)), 'Wo': _w((lambda *s: _rng.normal(s) * 0.05)(H, Dh, Dm) * (H * Dh) ** (-0.5)), 'seg_len': seg}
    _A_in = _A_setup()

    def _B_setup():
        B, S, D, F, C = (1, 2048, 640, 1728, 8)
        return {'x': _w((lambda *s: _rng.normal(s) * 0.05)(B, S, D)), 'w_r': _w((lambda *s: _rng.normal(s) * 0.05)(D)), 'w_gate': _w((lambda *s: _rng.normal(s) * 0.05)(D, F)), 'w_up': _w((lambda *s: _rng.normal(s) * 0.05)(D, F)), 'w_down': _w((lambda *s: _rng.normal(s) * 0.05)(F, D))}
    _B_in = _B_setup()
    return {'A_x': _A_in['x'], 'A_mem0': _A_in['mem0'], 'A_Wq': _A_in['Wq'], 'A_Wk': _A_in['Wk'], 'A_Wv': _A_in['Wv'], 'A_Wo': _A_in['Wo'], 'A_seg_len': _A_in['seg_len'], 'B_x': _B_in['x'], 'B_w_r': _B_in['w_r'], 'B_w_gate': _B_in['w_gate'], 'B_w_up': _B_in['w_up'], 'B_w_down': _B_in['w_down']}

def reference(A_x, A_mem0, A_Wq, A_Wk, A_Wv, A_Wo, A_seg_len, B_x, B_w_r, B_w_gate, B_w_up, B_w_down):

    def _A_ref(x, mem0, Wq, Wk, Wv, Wo, seg_len):
        B, S, Dm = x.shape
        H, Dh = (Wq.shape[1], Wq.shape[2])
        M = mem0.shape[1]
        scale = Dh ** (-0.5)
        n_seg = S // seg_len
        L = M + seg_len
        idx = jnp.arange(L)
        mask = (idx[:, None] < M) | (idx[:, None] >= idx[None, :])
        mem = mem0
        outs = []
        for s in range(n_seg):
            xs = x[:, s * seg_len:(s + 1) * seg_len, :].copy()
            h = jnp.concatenate([mem, xs], axis=1)
            q = jnp.einsum('btd,dhe->bhte', h, Wq)
            k = jnp.einsum('btd,dhe->bhte', h, Wk)
            v = jnp.einsum('btd,dhe->bhte', h, Wv)
            scores = jnp.einsum('bhqe,bhke->bhqk', q, k) * scale
            scores = jnp.where(mask[None, None], scores, -1000000000.0)
            p = _softmax(scores, axis=-1)
            o = jnp.einsum('bhqk,bhke->bhqe', p, v)
            o = jnp.einsum('bhte,hed->btd', o, Wo)
            mem = o[:, :M, :].copy()
            outs.append(o[:, M:, :])
        return jnp.concatenate(outs, axis=1)

    def _B_ref(x, w_r, w_gate, w_up, w_down):
        B, S, D = x.shape
        C = 8
        r = x @ w_r
        idx = jnp.argsort(-r, axis=-1)[:, :C]
        idx_e = jnp.repeat(idx.reshape(B, C, 1), D, axis=2)
        x_sel = jnp.take_along_axis(x, idx_e, axis=1)
        g = _silu(x_sel @ w_gate)
        u = x_sel @ w_up
        y = g * u @ w_down
        r_sel = _sigmoid(jnp.take_along_axis(r, idx, axis=1))
        y = y * r_sel.reshape(B, C, 1)
        b_off = (jnp.arange(B) * S).reshape(B, 1)
        flat_idx = (idx + b_off).reshape(B * C)
        zero = (x * 0.0).reshape(B * S, D)
        upd = _scatter_add(zero, flat_idx, y.reshape(B * C, D), axis=0)
        return x + upd.reshape(B, S, D)
    x = A_x
    xn = _layernorm(x, axis=-1)
    s = _A_ref(xn, A_mem0, A_Wq, A_Wk, A_Wv, A_Wo, A_seg_len)
    g = _silu(_B_ref(xn, B_w_r, B_w_gate, B_w_up, B_w_down))
    return x + s * g
```

```python
import functools

import jax
import jax.numpy as jnp
import numpy as np
from jax import lax
import jax.experimental.pallas as pl
import jax.experimental.pallas.tpu as pltpu

F32 = jnp.float32
BF16 = jnp.bfloat16
U32 = jnp.uint32
I32 = jnp.int32

TOP_C = 8
LANES = 128
PRE_ROWS = 8
N_PRE = 64
DBG_STEPS = 64
ORDER = 1
SCHED = 1
LAG_S = 2
LAG_P = 3
LN_ROWS = 256
EPS_BF16 = float(np.float32(1.0013580322265625e-05))

_NN = (((1,), (0,)), ((), ()))
_NT = (((1,), (1,)), ((), ()))


def _rb(x):
    return x.astype(BF16).astype(F32)


def _dot(a, b, dims=_NN):
    return lax.dot_general(a, b, dims, preferred_element_type=F32)


def _layernorm(xb):
    x = xb.astype(F32)
    inv_n = 1.0 / x.shape[-1]
    mean = jnp.sum(x, axis=-1, keepdims=True) * inv_n
    c = x - mean
    var = jnp.sum(c * c, axis=-1, keepdims=True) * inv_n
    sd = _rb(jnp.sqrt(_rb(_rb(var) + EPS_BF16)))
    return _rb(_rb(x - _rb(mean)) / sd)


def _sigmoid(x):
    return 1.0 / (1.0 + jnp.exp(-x))


def _silu(x):
    return _rb(x * _rb(_sigmoid(x)))


def _kernel(x_hbm, mem0_ref, wq_hbm, wk_hbm, wv_hbm, wo_hbm, wr_ref, wg_hbm, wu_hbm, wd_hbm,
            out_hbm,
            x_s, xn_s, g_s, xpre_s, raw_s, w_s, wo_s, wg_s, wu_s, wd_s, pre_s, r_s, out_s,
            sem_x, sem_w, sem_o, sem_f, sem_out, *, seg):
    S, D = x_s.shape
    H, E = wq_hbm.shape[1], wq_hbm.shape[2]
    M = mem0_ref.shape[0]
    n_seg = S // seg
    L = seg + M
    n_pair = 3 * H // 2
    n_col = D // LANES
    n_ln = S // LN_ROWS
    scale = E ** -0.5

    def x_copy(i):
        rows = pl.ds(i * LN_ROWS, LN_ROWS)
        return pltpu.make_async_copy(x_hbm.at[rows], x_s.at[rows], sem_x.at[i])

    def pair_start(m, c):
        src = (wq_hbm, wk_hbm, wv_hbm)[m].bitcast(U32).at[:, c, :]
        p = m * (H // 2) + c
        return pltpu.make_async_copy(src, raw_s.at[p], sem_w.at[p])

    def pair_wait(p):
        pltpu.make_async_copy(raw_s.at[p], raw_s.at[p], sem_w.at[p]).wait()

    def wo_copy(n):
        return pltpu.make_async_copy(wo_hbm.at[:, pl.ds(n * LANES, LANES)], wo_s.at[n], sem_o.at[n])

    ffn_copies = [pltpu.make_async_copy(src, dst, sem_f.at[i])
                  for i, (src, dst) in enumerate(((wg_hbm, wg_s), (wu_hbm, wu_s), (wd_hbm, wd_s)))]

    with jax.named_scope("issue"):
        for i in range(n_ln):
            x_copy(i).start()
        if ORDER == 0:
            for m in range(3):
                for c in range(H // 2):
                    pair_start(m, c).start()
            for n in range(n_col):
                wo_copy(n).start()
            for cp in ffn_copies:
                cp.start()
        if ORDER == 2:
            for m in range(3):
                for c in range(H // 2):
                    pair_start(m, c).start()

    wr = jnp.broadcast_to(wr_ref[...].astype(F32).reshape(1, D), (8, D))

    def ln_block(i, carry):
        x_copy(i).wait()
        r0 = pl.multiple_of(i * LN_ROWS, LN_ROWS)
        xn = _layernorm(x_s[pl.ds(r0, LN_ROWS), :])
        xn_s[pl.ds(r0, LN_ROWS), :] = xn
        g_s[pl.ds(r0, LN_ROWS), :] = _silu(xn + xn * 0.0)
        n_loc = LN_ROWS // seg
        pre = jnp.concatenate([xn[j * seg:j * seg + PRE_ROWS] for j in range(n_loc)], axis=0)
        p0 = pl.multiple_of(i * (n_loc * PRE_ROWS), n_loc * PRE_ROWS)
        xpre_s[pl.ds(p0, n_loc * PRE_ROWS), :] = pre.astype(BF16)
        r_s[i] = _dot(wr, xn.astype(BF16), _NT)
        return carry

    with jax.named_scope("ln"):
        lax.fori_loop(0, n_ln, ln_block, 0)
    if ORDER == 1:
        for m in range(3):
            for c in range(H // 2):
                pair_start(m, c).start()
    if ORDER >= 1:
        for n in range(n_col):
            wo_copy(n).start()
        for cp in ffn_copies:
            cp.start()

    idx_bits = (S - 1).bit_length()
    int_min = np.int32(-2 ** 31)
    sub = lax.broadcasted_iota(I32, (8, LN_ROWS), 0)
    r_all = jnp.zeros((8, LN_ROWS), F32)
    for i in range(n_ln):
        r_all = jnp.where(sub == i, r_s[i], r_all)
    r_all = _rb(r_all)
    r_all = jnp.where(r_all == 0.0, 0.0, r_all)
    bits = lax.bitcast_convert_type(r_all, I32) >> 16
    code = jnp.where(bits < 0, bits ^ 0x7FFF, bits)
    code = jnp.where(r_all != r_all, -32768, code)
    tok = sub * LN_ROWS + lax.broadcasted_iota(I32, (8, LN_ROWS), 1)
    keys = (code << idx_bits) | (S - 1 - tok)
    sel_idx = []
    r_sel = jnp.zeros((TOP_C, LANES), F32)
    row_c = lax.broadcasted_iota(I32, (TOP_C, LANES), 0)
    for c in range(TOP_C):
        best = jnp.max(keys)
        hit = keys == best
        sel_idx.append(S - 1 - (best & (2 ** idx_bits - 1)))
        val = jnp.sum(jnp.where(hit, r_all, 0.0), axis=1, keepdims=True)
        val = jnp.sum(val, axis=0, keepdims=True)
        r_sel = jnp.where(row_c == c, val, r_sel)
        keys = jnp.where(hit, int_min, keys)

    def repack(p):
        a = raw_s[p, pl.ds(0, D // 2, stride=2), :]
        b = raw_s[p, pl.ds(1, D // 2, stride=2), :]
        w_s[2 * p] = (a & np.uint32(0xFFFF)) | (b << 16)
        w_s[2 * p + 1] = (a >> 16) | (b & np.uint32(0xFFFF0000))

    def w_slab(i):
        return pltpu.bitcast(w_s[i], BF16)

    n_it = N_PRE // 4
    per_it = -(-(n_pair - 2) // n_it) if n_it else 0
    done = 0
    if n_it:
        for p in range(2):
            pair_wait(p)
            repack(p)
        n_full = min(n_it, (n_pair - 2) // per_it)

        def pre_iter(it, n_repack, first):
            for j in range(n_repack):
                pair_wait(first + j)
            for j in range(n_repack):
                repack(first + j)
            w4 = jnp.concatenate([w_slab(4 * it + j) for j in range(4)], axis=1)
            res = _dot(xpre_s[...], w4)
            for j in range(4):
                pre_s[4 * it + j] = res[:, j * E:(j + 1) * E]

        def pre_body(it, carry):
            pre_iter(it, per_it, 2 + it * per_it)
            return carry

        with jax.named_scope("pre"):
            lax.fori_loop(0, n_full, pre_body, 0)
        done = 2 + n_full * per_it
        for it in range(n_full, n_it):
            k = min(per_it, n_pair - done)
            pre_iter(it, k, done)
            done += k

    def tail_body(p, carry):
        pair_wait(p)
        repack(p)
        return carry

    with jax.named_scope("tail"):
        lax.fori_loop(done, n_pair, tail_body, 0)

    with jax.named_scope("ffnwait"):
        for cp in ffn_copies:
            cp.wait()
    x_sel = jnp.concatenate([xn_s[pl.ds(t, 1), :] for t in sel_idx], axis=0)
    gate = _silu(_rb(_dot(x_sel, wg_s[...], _NT)))
    up = _rb(_dot(x_sel, wu_s[...], _NT))
    y = _rb(_dot(_rb(gate * up), wd_s[...]))
    y = _rb(y * _rb(_sigmoid(r_sel[:, :1])))
    g_sel = _silu(_rb(x_sel + (x_sel * 0.0 + y)))
    for c, t in enumerate(sel_idx):
        g_s[pl.ds(t, 1), :] = g_sel[c:c + 1]
    for n in range(n_col):
        wo_copy(n).wait()

    hpg = LANES // L
    groups = [list(range(h, min(h + hpg, H))) for h in range(0, H, hpg)]
    lane = lax.broadcasted_iota(I32, (L, LANES), 1)
    key_j = lax.broadcasted_iota(I32, (L, LANES), 0)
    qry_t = lane
    for i in range(1, hpg):
        qry_t = jnp.where(lane >= i * L, lane - i * L, qry_t)
    allowed = (qry_t >= seg) | (key_j >= seg) | (key_j <= qry_t)

    def step(s, mem):
        r0 = pl.multiple_of(s * seg, seg)
        p0 = pl.multiple_of(s * PRE_ROWS, PRE_ROWS)
        h_all = jnp.concatenate([xn_s[pl.ds(r0, seg), :], mem], axis=0)
        h_rest = h_all[PRE_ROWS:].astype(BF16)

        def project(m, heads):
            ids = [m * H + h for h in heads]
            out = {}
            for is_pre in (True, False):
                sel = [i for i in ids if (i < N_PRE) == is_pre]
                if not sel:
                    continue
                w = jnp.concatenate([w_slab(i) for i in sel], axis=1)
                res = _dot(h_rest if is_pre else h_all, w)
                for j, i in enumerate(sel):
                    blk = res[:, j * E:(j + 1) * E]
                    if is_pre:
                        blk = jnp.concatenate([pre_s[i, pl.ds(p0, PRE_ROWS), :], blk], axis=0)
                    out[i] = blk
            return [out[i] for i in ids]

        def scores(q, k):
            n = len(q)
            qs = jnp.concatenate(q + [jnp.zeros((LANES - n * L, E), F32)], axis=0).astype(BF16)
            st = _dot(jnp.concatenate(k, axis=0), qs, _NT)
            merged = st[:L]
            for i in range(1, n):
                merged = jnp.where(lane >= i * L, st[i * L:(i + 1) * L], merged)
            sc = jnp.where(allowed, merged * scale, -1e9)
            e = jnp.exp(sc - jnp.max(sc, axis=0, keepdims=True))
            return e / jnp.sum(e, axis=0, keepdims=True)

        def mix(pt, v):
            p = jnp.concatenate([pt, jnp.zeros((LANES - L, LANES), F32)], axis=0).T
            outs = []
            for i, vh in enumerate(v):
                vp = jnp.concatenate([vh, jnp.zeros((LANES - L, E), F32)], axis=0).astype(BF16)
                outs.append(_dot(p[i * L:(i + 1) * L], vp))
            return outs

        n_g = len(groups)
        q, k, v, probs, o = {}, {}, {}, {}, {}
        if SCHED == 0:
            for g in range(n_g + LAG_S + LAG_P):
                if g < n_g:
                    q[g], k[g], v[g] = [project(m, groups[g]) for m in range(3)]
                gp = g - LAG_S - LAG_P
                if 0 <= gp < n_g:
                    o[gp] = mix(probs[gp], v[gp])
                gs = g - LAG_S
                if 0 <= gs < n_g:
                    probs[gs] = scores(q[gs], k[gs])
        elif SCHED == 1:
            work = [("qk", g) for g in range(n_g)] + [("v", g) for g in range(n_g)] + [("nop", 0)] * (LAG_P + LAG_S)
            for t, (kind, g) in enumerate(work):
                if kind == "qk":
                    q[g], k[g] = project(0, groups[g]), project(1, groups[g])
                elif kind == "v":
                    v[g] = project(2, groups[g])
                gs = t - LAG_S
                if 0 <= gs < n_g:
                    probs[gs] = scores(q[gs], k[gs])
                gp = t - n_g - LAG_P
                if 0 <= gp < n_g:
                    o[gp] = mix(probs[gp], v[gp])
        o = [oh for g in range(n_g) for oh in o[g]]

        o_all = jnp.concatenate([jnp.concatenate([oh[seg:], oh[:seg]], axis=0) for oh in o], axis=1)
        wo32 = wo_s.bitcast(U32)
        wo = jnp.concatenate([pltpu.bitcast(wo32[n], BF16) for n in range(n_col)], axis=1)
        res = _dot(o_all, wo)
        x = x_s[pl.ds(r0, seg), :].astype(F32)
        out = x + _rb(_rb(res[M:]) * g_s[pl.ds(r0, seg), :])
        out_s[pl.ds(r0, seg), :] = out.astype(BF16)
        pltpu.make_async_copy(out_s.at[pl.ds(r0, seg)], out_hbm.at[pl.ds(r0, seg)], sem_out).start()
        return res[:M]

    with jax.named_scope("main"):
        lax.fori_loop(0, DBG_STEPS, step, mem0_ref[...].astype(F32))
    pltpu.make_async_copy(out_s.at[pl.ds(0, DBG_STEPS * seg)], out_s.at[pl.ds(0, DBG_STEPS * seg)], sem_out).wait()


@functools.partial(jax.jit, static_argnames=("A_seg_len",))
def pallas_recurrent_scan__memory_aug_recurrent_mem_tr__moe_arch_mod__prompt_kernel(
    A_x: jax.Array,
    A_mem0: jax.Array,
    A_Wq: jax.Array,
    A_Wk: jax.Array,
    A_Wv: jax.Array,
    A_Wo: jax.Array,
    A_seg_len: int,
    B_x: jax.Array,
    B_w_r: jax.Array,
    B_w_gate: jax.Array,
    B_w_up: jax.Array,
    B_w_down: jax.Array,
):
    del B_x
    B, S, D = A_x.shape
    _, H, E = A_Wq.shape
    M = A_mem0.shape[1]
    Fh = B_w_gate.shape[1]
    seg = int(A_seg_len)
    n_seg = S // seg
    assert B == 1 and E == LANES and S % LN_ROWS == 0 and S // LN_ROWS == 8 and LN_ROWS % seg == 0

    hbm = pl.BlockSpec(memory_space=pltpu.HBM)
    vmem = pl.BlockSpec(memory_space=pltpu.VMEM)
    out = pl.pallas_call(
        functools.partial(_kernel, seg=seg),
        out_shape=jax.ShapeDtypeStruct((S, D), A_x.dtype),
        in_specs=[hbm, vmem, hbm, hbm, hbm, hbm, vmem, hbm, hbm, hbm],
        out_specs=hbm,
        scratch_shapes=[
            pltpu.VMEM((S, D), BF16),
            pltpu.VMEM((S, D), F32),
            pltpu.VMEM((S, D), F32),
            pltpu.VMEM((n_seg * PRE_ROWS, D), BF16),
            pltpu.VMEM((3 * H // 2, D, E), U32),
            pltpu.VMEM((3 * H, D // 2, E), U32),
            pltpu.VMEM((D // LANES, H * E, LANES), BF16),
            pltpu.VMEM((Fh, D), BF16),
            pltpu.VMEM((Fh, D), BF16),
            pltpu.VMEM((Fh, D), BF16),
            pltpu.VMEM((max(N_PRE, 1), n_seg * PRE_ROWS, E), F32),
            pltpu.VMEM((S // LN_ROWS, 8, LN_ROWS), F32),
            pltpu.VMEM((S, D), BF16),
            pltpu.SemaphoreType.DMA((S // LN_ROWS,)),
            pltpu.SemaphoreType.DMA((3 * H // 2,)),
            pltpu.SemaphoreType.DMA((D // LANES,)),
            pltpu.SemaphoreType.DMA((3,)),
            pltpu.SemaphoreType.DMA(()),
        ],
        compiler_params=pltpu.CompilerParams(vmem_limit_bytes=110 * 1024 * 1024),
    )(A_x.reshape(S, D), A_mem0.reshape(M, D), A_Wq, A_Wk, A_Wv, A_Wo.reshape(H * E, D),
      B_w_r, B_w_gate.T, B_w_up.T, B_w_down)
    return out.reshape(B, S, D)
```

```python
import functools

import jax
import jax.numpy as jnp
import numpy as np
from jax import lax
import jax.experimental.pallas as pl
import jax.experimental.pallas.tpu as pltpu

F32 = jnp.float32
BF16 = jnp.bfloat16
U32 = jnp.uint32
I32 = jnp.int32

TOP_C = 8
LANES = 128
PRE_ROWS = 8
N_BLK = 8
DBG_STEPS = 64
LAG_S = 2
LAG_P = 3
PRE_M = 64
LN_ROWS = 16
LN_END = 2
UNROLL = 4
CHUNK_PAIRS = 2

EPS_BF16 = float(np.float32(1.0013580322265625e-05))

_NN = (((1,), (0,)), ((), ()))
_NT = (((1,), (1,)), ((), ()))


def _rb(x):
    return x.astype(BF16).astype(F32)


def _dot(a, b, dims=_NN):
    return lax.dot_general(a, b, dims, preferred_element_type=F32)


def _layernorm(x):
    inv_n = 1.0 / x.shape[-1]
    mean = jnp.sum(x, axis=-1, keepdims=True) * inv_n
    c = x - mean
    var = jnp.sum(c * c, axis=-1, keepdims=True) * inv_n
    sd = _rb(jnp.sqrt(_rb(_rb(var) + EPS_BF16)))
    return _rb(_rb(x - _rb(mean)) * (1.0 / sd))


def _sigmoid(x):
    return 1.0 / (1.0 + jnp.exp(-x))


def _silu(x):
    return _rb(x * _rb(_sigmoid(x)))


def _kernel(x_hbm, mem0_ref, wq_hbm, wk_hbm, wv_hbm, wo_hbm, wr_ref, wg_hbm, wu_hbm, wd_hbm,
            out_hbm,
            x_s, xp_s, xpre_s, raw_s, w_s, wo_s, wg_s, wu_s, wd_s, act_s, r_s, out_s,
            sem, sem_out):
    n_seg, seg, D = x_hbm.shape
    S = n_seg * seg
    H, E = wq_hbm.shape[1], wq_hbm.shape[2]
    M = mem0_ref.shape[0]
    L = seg + M
    n_pair = 3 * H // 2
    n_col = D // LANES
    scale = E ** -0.5
    seg_blk = n_seg // N_BLK
    rows_blk = seg_blk * seg
    pair_blk = n_pair // N_BLK

    n_pre = n_seg * PRE_ROWS
    XN, GATE, PRE = 0, n_col * S, 2 * n_col * S

    def act_load(base, r, n, stride=S, tiles=n_col):
        return jnp.concatenate([act_s[pl.ds(base + c * stride + r, n), :] for c in range(tiles)],
                               axis=1)

    def act_store(base, r, val, stride=S):
        for c in range(val.shape[1] // LANES):
            act_s[pl.ds(base + c * stride + r, val.shape[0]), :] = val[:, c * LANES:(c + 1) * LANES]

    SEM_X, SEM_P = 1, 1 + N_BLK
    SEM_F = SEM_P + n_pair
    SEM_O = SEM_F + 3
    xp_copy = pltpu.make_async_copy(x_hbm.at[:, pl.ds(0, PRE_ROWS), :], xp_s, sem.at[0])

    def x_copy(i):
        blk = pl.ds(i * seg_blk, seg_blk)
        return pltpu.make_async_copy(x_hbm.at[blk], x_s.at[blk], sem.at[SEM_X + i])

    def pair_copy(p):
        m, c = divmod(p, H // 2)
        src = (wq_hbm, wk_hbm, wv_hbm)[m].bitcast(U32).at[:, c, :]
        return pltpu.make_async_copy(src, raw_s.at[p], sem.at[SEM_P + p])

    def pair_wait(p):
        pltpu.make_async_copy(raw_s.at[p], raw_s.at[p], sem.at[SEM_P + p]).wait()

    ffn_copies = [pltpu.make_async_copy(src, dst, sem.at[SEM_F + i])
                  for i, (src, dst) in enumerate(((wg_hbm, wg_s), (wu_hbm, wu_s), (wd_hbm, wd_s)))]
    wo_copies = [pltpu.make_async_copy(wo_hbm.at[:, pl.ds(n * LANES, LANES)], wo_s.at[n],
                                       sem.at[SEM_O + n]) for n in range(n_col)]

    xp_copy.start()
    for i in range(N_BLK):
        for p in range(i * pair_blk, (i + 1) * pair_blk):
            pair_copy(p).start()
        x_copy(i).start()
    for cp in ffn_copies + wo_copies:
        cp.start()

    with jax.named_scope("lnpre"):
        xp_copy.wait()
        xp = xp_s[...].astype(F32).reshape(n_seg * PRE_ROWS, D)
        xpre_s[...] = _layernorm(xp).astype(BF16)

    wr = wr_ref[...].astype(F32).reshape(1, D)
    lane8 = lax.broadcasted_iota(I32, (8, LANES), 1)

    def pre_block(it, carry):
        for j in range(pair_blk):
            pair_wait(it * pair_blk + j)
        x_copy(it).wait()
        n_rows = n_seg * PRE_ROWS
        n_piece = (pair_blk // CHUNK_PAIRS) * (n_rows // PRE_M)
        dense = jnp.zeros((8, LANES), F32)
        piece = done = 0
        for j in range(0, pair_blk, CHUNK_PAIRS):
            slabs = []
            for p in [it * pair_blk + j + jj for jj in range(CHUNK_PAIRS)]:
                a = raw_s[p, pl.ds(0, D // 2, stride=2), :]
                b = raw_s[p, pl.ds(1, D // 2, stride=2), :]
                lo = (a & np.uint32(0xFFFF)) | (b << 16)
                hi = (a >> 16) | (b & np.uint32(0xFFFF0000))
                w_s[2 * p] = lo
                w_s[2 * p + 1] = hi
                slabs += [pltpu.bitcast(lo, BF16), pltpu.bitcast(hi, BF16)]
            w = jnp.concatenate(slabs, axis=1)
            for mb in range(0, n_rows, PRE_M):
                res = _dot(xpre_s[mb:mb + PRE_M, :], w)
                act_store(PRE, pl.multiple_of(2 * (it * pair_blk + j) * n_pre + mb, PRE_M), res, n_pre)
                piece += 1
                n_ln = rows_blk // LN_ROWS
                while done < min(n_ln, -(-piece * n_ln // (n_piece - LN_END))):
                    sg, off = divmod(done * LN_ROWS, seg)
                    x = x_s[it * seg_blk + sg, off:off + LN_ROWS, :].astype(F32)
                    xn = _layernorm(x)
                    r0 = pl.multiple_of(it * rows_blk + done * LN_ROWS, LN_ROWS)
                    act_store(XN, r0, xn)
                    act_store(GATE, r0, _silu(xn + xn * 0.0))
                    score = jnp.sum(xn * wr, axis=-1, keepdims=True)
                    for r in range(LN_ROWS // 8):
                        dense = jnp.where(lane8 == done * (LN_ROWS // 8) + r,
                                          score[8 * r:8 * r + 8], dense)
                    done += 1
        r_s[it] = dense
        return carry

    with jax.named_scope("pre"):
        lax.fori_loop(0, N_BLK, pre_block, 0)

    idx_bits = (S - 1).bit_length()
    int_min = np.int32(-2 ** 31)
    r_all = _rb(r_s[...].reshape(N_BLK * 8, LANES))
    r_all = jnp.where(r_all == 0.0, 0.0, r_all)
    bits = lax.bitcast_convert_type(r_all, I32) >> 16
    code = jnp.where(bits < 0, bits ^ 0x7FFF, bits)
    code = jnp.where(r_all != r_all, -32768, code)
    row = lax.broadcasted_iota(I32, r_all.shape, 0)
    col = lax.broadcasted_iota(I32, r_all.shape, 1)
    tok = (row >> 3) * rows_blk + col * 8 + (row & 7)
    keys = jnp.where(col < rows_blk // 8, (code << idx_bits) | (S - 1 - tok), int_min)
    row_c = lax.broadcasted_iota(I32, (TOP_C, LANES), 0)
    best_keys = jnp.zeros((TOP_C, LANES), I32)
    for c in range(TOP_C):
        best = jnp.max(jnp.max(keys, axis=0, keepdims=True), axis=1, keepdims=True)
        best_keys = jnp.where(row_c == c, best, best_keys)
        keys = jnp.where(keys == best, int_min, keys)
    best_code = best_keys >> idx_bits
    r_sel = lax.bitcast_convert_type(
        jnp.where(best_code < 0, best_code ^ 0x7FFF, best_code) << 16, F32)
    best_tok = S - 1 - (best_keys & (2 ** idx_bits - 1))
    sel_idx = [jnp.max(jnp.where(row_c == c, best_tok, 0)) for c in range(TOP_C)]

    with jax.named_scope("ffnwait"):
        for cp in ffn_copies:
            cp.wait()
    x_sel = jnp.concatenate([act_load(XN, t, 1) for t in sel_idx], axis=0)
    gate = _silu(_rb(_dot(x_sel, wg_s[...], _NT)))
    up = _rb(_dot(x_sel, wu_s[...], _NT))
    y = _rb(_dot(_rb(gate * up), wd_s[...]))
    y = _rb(y * _rb(_sigmoid(r_sel[:, :1])))
    g_sel = _silu(_rb(x_sel + (x_sel * 0.0 + y)))
    for c, t in enumerate(sel_idx):
        act_store(GATE, t, g_sel[c:c + 1])
    with jax.named_scope("wowait"):
        for cp in wo_copies:
            cp.wait()

    hpg = LANES // L
    groups = [list(range(h, min(h + hpg, H))) for h in range(0, H, hpg)]
    lane = lax.broadcasted_iota(I32, (L, LANES), 1)
    key_j = lax.broadcasted_iota(I32, (L, LANES), 0)
    qry_t = lane
    for i in range(1, hpg):
        qry_t = jnp.where(lane >= i * L, lane - i * L, qry_t)
    allowed = (qry_t >= seg) | (key_j >= seg) | (key_j <= qry_t)

    def step(s, mem):
        r0 = pl.multiple_of(s * seg, seg)
        p0 = pl.multiple_of(s * PRE_ROWS, PRE_ROWS)
        h_rest = jnp.concatenate(
            [act_load(XN + PRE_ROWS, r0, seg - PRE_ROWS), mem], axis=0).astype(BF16)

        def project(m, heads):
            ids = [m * H + h for h in heads]
            w = jnp.concatenate([pltpu.bitcast(w_s[i], BF16) for i in ids], axis=1)
            res = _dot(h_rest, w)
            return [jnp.concatenate([act_s[pl.ds(PRE + i * n_pre + p0, PRE_ROWS), :], res[:, j * E:(j + 1) * E]],
                                    axis=0) for j, i in enumerate(ids)]

        def scores(q, k):
            n = len(q)
            qs = jnp.concatenate(q + [jnp.zeros((LANES - n * L, E), F32)], axis=0).astype(BF16)
            st = _dot(jnp.concatenate(k, axis=0), qs, _NT)
            merged = st[:L]
            for i in range(1, n):
                merged = jnp.where(lane >= i * L, st[i * L:(i + 1) * L], merged)
            sc = jnp.where(allowed, merged * scale, -1e9)
            e = jnp.exp(sc - jnp.max(sc, axis=0, keepdims=True))
            return e / jnp.sum(e, axis=0, keepdims=True)

        def mix(pt, v):
            p = jnp.concatenate([pt, jnp.zeros((LANES - L, LANES), F32)], axis=0).T
            outs = []
            for i, vh in enumerate(v):
                vp = jnp.concatenate([vh, jnp.zeros((LANES - L, E), F32)], axis=0).astype(BF16)
                outs.append(_dot(p[i * L:(i + 1) * L], vp))
            return outs

        n_g = len(groups)
        q, k, v, probs, o = {}, {}, {}, {}, {}
        for t in range(2 * n_g + LAG_P):
            if t < n_g:
                q[t], k[t] = project(0, groups[t]), project(1, groups[t])
            elif t < 2 * n_g:
                v[t - n_g] = project(2, groups[t - n_g])
            gs = t - LAG_S
            if 0 <= gs < n_g:
                probs[gs] = scores(q[gs], k[gs])
            gp = t - n_g - LAG_P
            if 0 <= gp < n_g:
                o[gp] = mix(probs[gp], v[gp])
        o = [oh for g in range(n_g) for oh in o[g]]

        o_all = jnp.concatenate([jnp.concatenate([oh[seg:], oh[:seg]], axis=0) for oh in o], axis=1)
        wo32 = wo_s.bitcast(U32)
        wo = jnp.concatenate([pltpu.bitcast(wo32[n], BF16) for n in range(n_col)], axis=1)
        res = _dot(o_all, wo)
        out = x_s[s].astype(F32) + _rb(_rb(res[M:]) * act_load(GATE, r0, seg))
        out_s[s] = out.astype(BF16)
        pltpu.make_async_copy(out_s.at[s], out_hbm.at[s], sem_out).start()
        return res[:M]

    with jax.named_scope("main"):
        lax.fori_loop(0, DBG_STEPS, step, mem0_ref[...].astype(F32), unroll=UNROLL)
    done = out_s.at[pl.ds(0, DBG_STEPS)]
    pltpu.make_async_copy(done, done, sem_out).wait()


@functools.partial(jax.jit, static_argnames=("A_seg_len",))
def pallas_recurrent_scan__memory_aug_recurrent_mem_tr__moe_arch_mod__prompt_kernel(
    A_x: jax.Array,
    A_mem0: jax.Array,
    A_Wq: jax.Array,
    A_Wk: jax.Array,
    A_Wv: jax.Array,
    A_Wo: jax.Array,
    A_seg_len: int,
    B_x: jax.Array,
    B_w_r: jax.Array,
    B_w_gate: jax.Array,
    B_w_up: jax.Array,
    B_w_down: jax.Array,
):
    del B_x
    B, S, D = A_x.shape
    _, H, E = A_Wq.shape
    M = A_mem0.shape[1]
    Fh = B_w_gate.shape[1]
    seg = int(A_seg_len)
    n_seg = S // seg

    hbm = pl.BlockSpec(memory_space=pltpu.HBM)
    vmem = pl.BlockSpec(memory_space=pltpu.VMEM)
    out = pl.pallas_call(
        _kernel,
        out_shape=jax.ShapeDtypeStruct((n_seg, seg, D), A_x.dtype),
        in_specs=[hbm, vmem, hbm, hbm, hbm, hbm, vmem, hbm, hbm, hbm],
        out_specs=hbm,
        scratch_shapes=[
            pltpu.VMEM((n_seg, seg, D), BF16),
            pltpu.VMEM((n_seg, PRE_ROWS, D), BF16),
            pltpu.VMEM((n_seg * PRE_ROWS, D), BF16),
            pltpu.VMEM((3 * H // 2, D, E), U32),
            pltpu.VMEM((3 * H, D // 2, E), U32),
            pltpu.VMEM((D // LANES, H * E, LANES), BF16),
            pltpu.VMEM((Fh, D), BF16),
            pltpu.VMEM((Fh, D), BF16),
            pltpu.VMEM((Fh, D), BF16),
            pltpu.VMEM((2 * (D // LANES) * S + 3 * H * n_seg * PRE_ROWS, LANES), F32),
            pltpu.VMEM((N_BLK, 8, LANES), F32),
            pltpu.VMEM((n_seg, seg, D), BF16),
            pltpu.SemaphoreType.DMA((1 + N_BLK + 3 * H // 2 + 3 + D // LANES,)),
            pltpu.SemaphoreType.DMA(()),
        ],
        compiler_params=pltpu.CompilerParams(vmem_limit_bytes=110 * 1024 * 1024),
    )(A_x.reshape(n_seg, seg, D), A_mem0.reshape(M, D), A_Wq, A_Wk, A_Wv, A_Wo.reshape(H * E, D),
      B_w_r, B_w_gate.T, B_w_up.T, B_w_down)
    return out.reshape(B, S, D)
```

```python
import functools

import jax
import jax.numpy as jnp
import numpy as np
from jax import lax
import jax.experimental.pallas as pl
import jax.experimental.pallas.tpu as pltpu

F32 = jnp.float32
BF16 = jnp.bfloat16
U32 = jnp.uint32
I32 = jnp.int32

TOP_C = 8
LANES = 128
PRE_ROWS = 8
N_BLK = 8
DBG_STEPS = 64
LAG_S = 3
LAG_P = 3
PRE_M = 64
LN_ROWS = 16
LN_END = 2
UNROLL = 8
N_SPLIT = 1
CHUNK_PAIRS = 2

EPS_BF16 = float(np.float32(1.0013580322265625e-05))

_NN = (((1,), (0,)), ((), ()))
_NT = (((1,), (1,)), ((), ()))


def _rb(x):
    return x.astype(BF16).astype(F32)


def _dot(a, b, dims=_NN):
    return lax.dot_general(a, b, dims, preferred_element_type=F32)


def _layernorm(x):
    inv_n = 1.0 / x.shape[-1]
    mean = jnp.sum(x, axis=-1, keepdims=True) * inv_n
    c = x - mean
    var = jnp.sum(c * c, axis=-1, keepdims=True) * inv_n
    sd = _rb(jnp.sqrt(_rb(_rb(var) + EPS_BF16)))
    return _rb(_rb(x - _rb(mean)) * (1.0 / sd))


def _sigmoid(x):
    return 1.0 / (1.0 + jnp.exp(-x))


def _silu(x):
    return _rb(x * _rb(_sigmoid(x)))


def _kernel(x_hbm, mem0_ref, wq_hbm, wk_hbm, wv_hbm, wo_hbm, wr_ref, wg_hbm, wu_hbm, wd_hbm,
            out_hbm,
            x_s, xp_s, xpre_s, raw_s, w_s, wo_s, wg_s, wu_s, wd_s, act_s, r_s, out_s,
            sem, sem_out):
    n_seg, seg, D = x_hbm.shape
    S = n_seg * seg
    H, E = wq_hbm.shape[1], wq_hbm.shape[2]
    M = mem0_ref.shape[0]
    L = seg + M
    n_pair = 3 * H // 2
    n_col = D // LANES
    scale = E ** -0.5
    seg_blk = n_seg // N_BLK
    rows_blk = seg_blk * seg
    pair_blk = n_pair // N_BLK

    n_pre = n_seg * PRE_ROWS
    XN, GATE, PRE = 0, n_col * S, 2 * n_col * S

    def act_load(base, r, n, stride=S, tiles=n_col):
        return jnp.concatenate([act_s[pl.ds(base + c * stride + r, n), :] for c in range(tiles)],
                               axis=1)

    def act_store(base, r, val, stride=S):
        for c in range(val.shape[1] // LANES):
            act_s[pl.ds(base + c * stride + r, val.shape[0]), :] = val[:, c * LANES:(c + 1) * LANES]

    SEM_X, SEM_P = 1, 1 + N_BLK
    SEM_F = SEM_P + n_pair
    SEM_O = SEM_F + 3
    xp_copy = pltpu.make_async_copy(x_hbm.at[:, pl.ds(0, PRE_ROWS), :], xp_s, sem.at[0])

    def x_copy(i):
        blk = pl.ds(i * seg_blk, seg_blk)
        return pltpu.make_async_copy(x_hbm.at[blk], x_s.at[blk], sem.at[SEM_X + i])

    def pair_copy(p):
        m, c = divmod(p, H // 2)
        src = (wq_hbm, wk_hbm, wv_hbm)[m].bitcast(U32).at[:, c, :]
        return pltpu.make_async_copy(src, raw_s.at[p], sem.at[SEM_P + p])

    def pair_wait(p):
        pltpu.make_async_copy(raw_s.at[p], raw_s.at[p], sem.at[SEM_P + p]).wait()

    ffn_copies = [pltpu.make_async_copy(src, dst, sem.at[SEM_F + i])
                  for i, (src, dst) in enumerate(((wg_hbm, wg_s), (wu_hbm, wu_s), (wd_hbm, wd_s)))]
    wo_copies = [pltpu.make_async_copy(wo_hbm.at[:, pl.ds(n * LANES, LANES)], wo_s.at[n],
                                       sem.at[SEM_O + n]) for n in range(n_col)]

    xp_copy.start()
    for i in range(N_BLK):
        for p in range(i * pair_blk, (i + 1) * pair_blk):
            pair_copy(p).start()
        x_copy(i).start()
    for cp in ffn_copies + wo_copies:
        cp.start()

    with jax.named_scope("lnpre"):
        xp_copy.wait()
        xp = xp_s[...].astype(F32).reshape(n_seg * PRE_ROWS, D)
        xpre_s[...] = _layernorm(xp).astype(BF16)

    wr = wr_ref[...].astype(F32).reshape(1, D)
    lane8 = lax.broadcasted_iota(I32, (8, LANES), 1)

    def pre_block(it, carry):
        for j in range(pair_blk):
            pair_wait(it * pair_blk + j)
        x_copy(it).wait()
        n_rows = n_seg * PRE_ROWS
        n_piece = (pair_blk // CHUNK_PAIRS) * (n_rows // PRE_M)
        dense = jnp.zeros((8, LANES), F32)
        piece = done = 0
        for j in range(0, pair_blk, CHUNK_PAIRS):
            slabs = []
            for p in [it * pair_blk + j + jj for jj in range(CHUNK_PAIRS)]:
                a = raw_s[p, pl.ds(0, D // 2, stride=2), :]
                b = raw_s[p, pl.ds(1, D // 2, stride=2), :]
                lo = (a & np.uint32(0xFFFF)) | (b << 16)
                hi = (a >> 16) | (b & np.uint32(0xFFFF0000))
                w_s[2 * p] = lo
                w_s[2 * p + 1] = hi
                slabs += [pltpu.bitcast(lo, BF16), pltpu.bitcast(hi, BF16)]
            w = jnp.concatenate(slabs, axis=1)
            for mb in range(0, n_rows, PRE_M):
                res = _dot(xpre_s[mb:mb + PRE_M, :], w)
                act_store(PRE, pl.multiple_of(2 * (it * pair_blk + j) * n_pre + mb, PRE_M), res, n_pre)
                piece += 1
                n_ln = rows_blk // LN_ROWS
                while done < min(n_ln, -(-piece * n_ln // (n_piece - LN_END))):
                    sg, off = divmod(done * LN_ROWS, seg)
                    x = x_s[it * seg_blk + sg, off:off + LN_ROWS, :].astype(F32)
                    xn = _layernorm(x)
                    r0 = pl.multiple_of(it * rows_blk + done * LN_ROWS, LN_ROWS)
                    act_store(XN, r0, xn)
                    act_store(GATE, r0, _silu(xn + xn * 0.0))
                    score = jnp.sum(xn * wr, axis=-1, keepdims=True)
                    for r in range(LN_ROWS // 8):
                        dense = jnp.where(lane8 == done * (LN_ROWS // 8) + r,
                                          score[8 * r:8 * r + 8], dense)
                    done += 1
        r_s[it] = dense
        return carry

    with jax.named_scope("pre"):
        lax.fori_loop(0, N_BLK, pre_block, 0)

    idx_bits = (S - 1).bit_length()
    int_min = np.int32(-2 ** 31)
    r_all = _rb(r_s[...].reshape(N_BLK * 8, LANES))
    r_all = jnp.where(r_all == 0.0, 0.0, r_all)
    bits = lax.bitcast_convert_type(r_all, I32) >> 16
    code = jnp.where(bits < 0, bits ^ 0x7FFF, bits)
    code = jnp.where(r_all != r_all, -32768, code)
    row = lax.broadcasted_iota(I32, r_all.shape, 0)
    col = lax.broadcasted_iota(I32, r_all.shape, 1)
    tok = (row >> 3) * rows_blk + col * 8 + (row & 7)
    keys = jnp.where(col < rows_blk // 8, (code << idx_bits) | (S - 1 - tok), int_min)
    row_c = lax.broadcasted_iota(I32, (TOP_C, LANES), 0)
    best_keys = jnp.zeros((TOP_C, LANES), I32)
    for c in range(TOP_C):
        best = jnp.max(jnp.max(keys, axis=0, keepdims=True), axis=1, keepdims=True)
        best_keys = jnp.where(row_c == c, best, best_keys)
        keys = jnp.where(keys == best, int_min, keys)
    best_code = best_keys >> idx_bits
    r_sel = lax.bitcast_convert_type(
        jnp.where(best_code < 0, best_code ^ 0x7FFF, best_code) << 16, F32)
    best_tok = S - 1 - (best_keys & (2 ** idx_bits - 1))
    sel_idx = [jnp.max(jnp.where(row_c == c, best_tok, 0)) for c in range(TOP_C)]

    with jax.named_scope("ffnwait"):
        for cp in ffn_copies:
            cp.wait()
    x_sel = jnp.concatenate([act_load(XN, t, 1) for t in sel_idx], axis=0)
    gate = _silu(_rb(_dot(x_sel, wg_s[...], _NT)))
    up = _rb(_dot(x_sel, wu_s[...], _NT))
    y = _rb(_dot(_rb(gate * up), wd_s[...]))
    y = _rb(y * _rb(_sigmoid(r_sel[:, :1])))
    g_sel = _silu(_rb(x_sel + (x_sel * 0.0 + y)))
    for c, t in enumerate(sel_idx):
        act_store(GATE, t, g_sel[c:c + 1])
    with jax.named_scope("wowait"):
        for cp in wo_copies:
            cp.wait()

    hpg = LANES // L
    groups = [list(range(h, min(h + hpg, H))) for h in range(0, H, hpg)]
    lane = lax.broadcasted_iota(I32, (L, LANES), 1)
    key_j = lax.broadcasted_iota(I32, (L, LANES), 0)
    qry_t = lane
    for i in range(1, hpg):
        qry_t = jnp.where(lane >= i * L, lane - i * L, qry_t)
    allowed = (qry_t >= seg) | (key_j >= seg) | (key_j <= qry_t)

    def step(s, mem):
        r0 = pl.multiple_of(s * seg, seg)
        p0 = pl.multiple_of(s * PRE_ROWS, PRE_ROWS)
        h_rest = jnp.concatenate(
            [act_load(XN + PRE_ROWS, r0, seg - PRE_ROWS), mem], axis=0).astype(BF16)

        def project(m, heads, k0=0, k1=D):
            w = jnp.concatenate(
                [pltpu.bitcast(w_s[m * H + h, k0 // 2:k1 // 2, :], BF16) for h in heads], axis=1)
            return _dot(h_rest[:, k0:k1], w)

        def with_early(m, heads, res):
            return [jnp.concatenate([act_s[pl.ds(PRE + (m * H + h) * n_pre + p0, PRE_ROWS), :],
                                     res[:, j * E:(j + 1) * E]], axis=0)
                    for j, h in enumerate(heads)]

        def scores(q, k):
            n = len(q)
            qs = jnp.concatenate(q + [jnp.zeros((LANES - n * L, E), F32)], axis=0).astype(BF16)
            st = _dot(jnp.concatenate(k, axis=0), qs, _NT)
            merged = st[:L]
            for i in range(1, n):
                merged = jnp.where(lane >= i * L, st[i * L:(i + 1) * L], merged)
            sc = jnp.where(allowed, merged * scale, -1e9)
            e = jnp.exp(sc - jnp.max(sc, axis=0, keepdims=True))
            return e / jnp.sum(e, axis=0, keepdims=True)

        def mix(pt, v):
            p = jnp.concatenate([pt, jnp.zeros((LANES - L, LANES), F32)], axis=0).T
            outs = []
            for i, vh in enumerate(v):
                vp = jnp.concatenate([vh, jnp.zeros((LANES - L, E), F32)], axis=0).astype(BF16)
                outs.append(_dot(p[i * L:(i + 1) * L], vp))
            return outs

        n_g = len(groups)
        wo32 = wo_s.bitcast(U32)

        def out_proj(n, outs, h0):
            lhs = jnp.concatenate(
                [jnp.concatenate([oh[seg:], oh[:seg]], axis=0) for oh in outs], axis=1)
            rows = slice(h0 * E // 2, (h0 + len(outs)) * E // 2)
            return _dot(lhs, pltpu.bitcast(wo32[n, rows, :], BF16))

        q, k, v, probs, o = {}, {}, {}, {}, {}
        k_split = D - LANES
        head_start = {(m, g): project(m, groups[g], 0, k_split)
                      for g in range(N_SPLIT) for m in range(2)}
        for t in range(2 * n_g):
            if t < n_g:
                for m, dst in ((0, q), (1, k)):
                    if (m, t) in head_start:
                        res = project(m, groups[t], k_split, D) + head_start[m, t]
                    else:
                        res = project(m, groups[t])
                    dst[t] = with_early(m, groups[t], res)
            else:
                v[t - n_g] = with_early(2, groups[t - n_g], project(2, groups[t - n_g]))
            gs = t - LAG_S
            if 0 <= gs < n_g:
                probs[gs] = scores(q[gs], k[gs])
            gp = t - n_g - LAG_P
            if 0 <= gp < n_g:
                o[gp] = mix(probs[gp], v[gp])
        n_early = n_g - LAG_P
        early = [oh for g in range(n_early) for oh in o[g]]
        col0 = None
        cuts = [len(early) * i // LAG_P for i in range(LAG_P + 1)]
        for i in range(LAG_P):
            part = out_proj(0, early[cuts[i]:cuts[i + 1]], cuts[i])
            col0 = part if col0 is None else part + col0
            o[n_early + i] = mix(probs[n_early + i], v[n_early + i])
        late = [oh for g in range(n_early, n_g) for oh in o[g]]
        cols = [None] + [out_proj(1, early + late, 0)]
        cols[0] = out_proj(0, late, len(early)) + col0
        cols += [out_proj(n, early + late, 0) for n in range(2, n_col)]
        res = jnp.concatenate(cols, axis=1)
        out = x_s[s].astype(F32) + _rb(_rb(res[M:]) * act_load(GATE, r0, seg))
        out_s[s] = out.astype(BF16)
        pltpu.make_async_copy(out_s.at[s], out_hbm.at[s], sem_out).start()
        return res[:M]

    with jax.named_scope("main"):
        lax.fori_loop(0, DBG_STEPS, step, mem0_ref[...].astype(F32), unroll=UNROLL)
    done = out_s.at[pl.ds(0, DBG_STEPS)]
    pltpu.make_async_copy(done, done, sem_out).wait()


@functools.partial(jax.jit, static_argnames=("A_seg_len",))
def pallas_recurrent_scan__memory_aug_recurrent_mem_tr__moe_arch_mod__prompt_kernel(
    A_x: jax.Array,
    A_mem0: jax.Array,
    A_Wq: jax.Array,
    A_Wk: jax.Array,
    A_Wv: jax.Array,
    A_Wo: jax.Array,
    A_seg_len: int,
    B_x: jax.Array,
    B_w_r: jax.Array,
    B_w_gate: jax.Array,
    B_w_up: jax.Array,
    B_w_down: jax.Array,
):
    del B_x
    B, S, D = A_x.shape
    _, H, E = A_Wq.shape
    M = A_mem0.shape[1]
    Fh = B_w_gate.shape[1]
    seg = int(A_seg_len)
    n_seg = S // seg

    hbm = pl.BlockSpec(memory_space=pltpu.HBM)
    vmem = pl.BlockSpec(memory_space=pltpu.VMEM)
    out = pl.pallas_call(
        _kernel,
        out_shape=jax.ShapeDtypeStruct((n_seg, seg, D), A_x.dtype),
        in_specs=[hbm, vmem, hbm, hbm, hbm, hbm, vmem, hbm, hbm, hbm],
        out_specs=hbm,
        scratch_shapes=[
            pltpu.VMEM((n_seg, seg, D), BF16),
            pltpu.VMEM((n_seg, PRE_ROWS, D), BF16),
            pltpu.VMEM((n_seg * PRE_ROWS, D), BF16),
            pltpu.VMEM((3 * H // 2, D, E), U32),
            pltpu.VMEM((3 * H, D // 2, E), U32),
            pltpu.VMEM((D // LANES, H * E, LANES), BF16),
            pltpu.VMEM((Fh, D), BF16),
            pltpu.VMEM((Fh, D), BF16),
            pltpu.VMEM((Fh, D), BF16),
            pltpu.VMEM((2 * (D // LANES) * S + 3 * H * n_seg * PRE_ROWS, LANES), F32),
            pltpu.VMEM((N_BLK, 8, LANES), F32),
            pltpu.VMEM((n_seg, seg, D), BF16),
            pltpu.SemaphoreType.DMA((1 + N_BLK + 3 * H // 2 + 3 + D // LANES,)),
            pltpu.SemaphoreType.DMA(()),
        ],
        compiler_params=pltpu.CompilerParams(vmem_limit_bytes=110 * 1024 * 1024),
    )(A_x.reshape(n_seg, seg, D), A_mem0.reshape(M, D), A_Wq, A_Wk, A_Wv, A_Wo.reshape(H * E, D),
      B_w_r, B_w_gate.T, B_w_up.T, B_w_down)
    return out.reshape(B, S, D)
```

```python
import functools

import jax
import jax.numpy as jnp
import numpy as np
from jax import lax
import jax.experimental.pallas as pl
import jax.experimental.pallas.tpu as pltpu

F32 = jnp.float32
BF16 = jnp.bfloat16
U32 = jnp.uint32
I32 = jnp.int32

TOP_C = 8
LANES = 128
PRE_ROWS = 8
N_BLK = 8
DBG_STEPS = 64
LAG_S = 3
LAG_P = 3
PRE_M = 64
FIRST = (2, 2)
LAST = 4
LNPRE_IT = 1
LN_ROWS = 8
SIDE_END = 2
FFN_W0 = 8
FFN_COLS = 256
UNROLL = 4
N_SPLIT = 1
CHUNK_PAIRS = 1

EPS_BF16 = float(np.float32(1.0013580322265625e-05))

_NN = (((1,), (0,)), ((), ()))
_NT = (((1,), (1,)), ((), ()))


def _rb(x):
    return x.astype(BF16).astype(F32)


def _dot(a, b, dims=_NN):
    return lax.dot_general(a, b, dims, preferred_element_type=F32)


def _layernorm(x):
    inv_n = 1.0 / x.shape[-1]
    mean = jnp.sum(x, axis=-1, keepdims=True) * inv_n
    c = x - mean
    var = jnp.sum(c * c, axis=-1, keepdims=True) * inv_n
    sd = _rb(jnp.sqrt(_rb(_rb(var) + EPS_BF16)))
    return _rb(_rb(x - _rb(mean)) * (1.0 / sd))


def _sigmoid(x):
    return 1.0 / (1.0 + jnp.exp(-x))


def _silu(x):
    return x * _sigmoid(x)


def _kernel(x_hbm, mem0_ref, wq_hbm, wk_hbm, wv_hbm, wo_hbm, wr_ref, wg_hbm, wu_hbm, wd_hbm,
            out_hbm,
            x_s, xp_s, xpre_s, raw_s, w_s, wo_s, wg_s, wu_s, wd_s, act_s, r_s, out_s,
            sem, sem_out):
    n_seg, seg, D = x_hbm.shape
    S = n_seg * seg
    H, E = wq_hbm.shape[1], wq_hbm.shape[2]
    M = mem0_ref.shape[0]
    L = seg + M
    n_pair = 3 * H // 2
    n_col = D // LANES
    scale = E ** -0.5
    seg_blk = n_seg // N_BLK
    rows_blk = seg_blk * seg
    pair_blk = (n_pair - sum(FIRST) - LAST) // N_BLK
    assert sum(FIRST) + N_BLK * pair_blk + LAST == n_pair

    n_pre = n_seg * PRE_ROWS
    XN, GATE, PRE = 0, n_col * S, 2 * n_col * S

    def act_load(base, r, n, stride=S, tiles=n_col):
        return jnp.concatenate([act_s[pl.ds(base + c * stride + r, n), :] for c in range(tiles)],
                               axis=1)

    def act_store(base, r, val, stride=S):
        for c in range(val.shape[1] // LANES):
            act_s[pl.ds(base + c * stride + r, val.shape[0]), :] = val[:, c * LANES:(c + 1) * LANES]

    SEM_XP, SEM_FIRST = 0, 1
    SEM_BLK = SEM_FIRST + len(FIRST)
    SEM_LAST, SEM_WO = SEM_BLK + N_BLK, SEM_BLK + N_BLK + 1
    xp_copy = pltpu.make_async_copy(x_hbm.at[:, pl.ds(0, PRE_ROWS), :], xp_s, sem.at[SEM_XP])

    def x_copy(i, n, sem_id):
        blk = pl.ds(i * seg_blk, n * seg_blk)
        return pltpu.make_async_copy(x_hbm.at[blk], x_s.at[blk], sem.at[sem_id])

    def pair_copy(p, sem_id):
        m, c = divmod(p, H // 2)
        src = (wq_hbm, wk_hbm, wv_hbm)[m].bitcast(U32).at[:, c, :]
        return pltpu.make_async_copy(src, raw_s.at[p], sem.at[sem_id])

    def pairs_wait(p, n, sem_id):
        dst = raw_s.at[pl.ds(p, n)]
        pltpu.make_async_copy(dst, dst, sem.at[sem_id]).wait()

    ffn_copies = [pltpu.make_async_copy(src, dst, sem.at[SEM_LAST])
                  for src, dst in ((wg_hbm, wg_s), (wu_hbm, wu_s), (wd_hbm, wd_s))]
    wo_copies = [pltpu.make_async_copy(wo_hbm.at[:, pl.ds(n * LANES, LANES)], wo_s.at[n],
                                       sem.at[SEM_WO]) for n in range(n_col)]

    xp_copy.start()
    p = 0
    for i, n in enumerate(FIRST):
        for _ in range(n):
            pair_copy(p, SEM_FIRST + i).start()
            p += 1
    for i in range(N_BLK):
        for _ in range(pair_blk):
            pair_copy(p, SEM_BLK + i).start()
            p += 1
        x_copy(i, 1, SEM_BLK + i).start()
    for _ in range(LAST):
        pair_copy(p, SEM_LAST).start()
        p += 1
    for cp in ffn_copies + wo_copies:
        cp.start()

    wr = wr_ref[...].astype(F32).reshape(1, D)
    lane8 = lax.broadcasted_iota(I32, (8, LANES), 1)

    def project_early(p_first, n_pairs, side_work):
        n_piece = (n_pairs // CHUNK_PAIRS) * (n_pre // PRE_M)
        piece = done = 0
        for j in range(0, n_pairs, CHUNK_PAIRS):
            slabs = []
            for p in [p_first + j + jj for jj in range(CHUNK_PAIRS)]:
                even = raw_s[p, pl.ds(0, D // 2, stride=2), :]
                odd = raw_s[p, pl.ds(1, D // 2, stride=2), :]
                lo = (even & np.uint32(0xFFFF)) | (odd << 16)
                hi = (even >> 16) | (odd & np.uint32(0xFFFF0000))
                w_s[2 * p] = lo
                w_s[2 * p + 1] = hi
                slabs += [pltpu.bitcast(lo, BF16), pltpu.bitcast(hi, BF16)]
            w = jnp.concatenate(slabs, axis=1)
            for mb in range(0, n_pre, PRE_M):
                res = _dot(xpre_s[mb:mb + PRE_M, :], w)
                r0 = 2 * (p_first + j) * n_pre + mb
                act_store(PRE, r0 if isinstance(r0, int) else pl.multiple_of(r0, PRE_M), res, n_pre)
                piece += 1
                while done < min(len(side_work),
                                 -(-piece * len(side_work) // (n_piece - SIDE_END))):
                    side_work[done]()
                    done += 1

    def norm_work(blk):
        dense = [jnp.zeros((8, LANES), F32)]

        def piece(i):
            sg, off = divmod(i * LN_ROWS, seg)
            xn = _layernorm(x_s[blk * seg_blk + sg, off:off + LN_ROWS, :].astype(F32))
            r0 = blk * rows_blk + i * LN_ROWS
            r0 = r0 if isinstance(r0, int) else pl.multiple_of(r0, LN_ROWS)
            act_store(XN, r0, xn)
            act_store(GATE, r0, _silu(xn + xn * 0.0))
            score = jnp.sum(xn * wr, axis=-1, keepdims=True)
            for r in range(LN_ROWS // 8):
                dense[0] = jnp.where(lane8 == i * (LN_ROWS // 8) + r, score[8 * r:8 * r + 8],
                                     dense[0])
            if (i + 1) * LN_ROWS == rows_blk:
                r_s[blk] = dense[0]

        return [functools.partial(piece, i) for i in range(rows_blk // LN_ROWS)]

    def routed_ffn_work():
        st = {}

        def select():
            idx_bits = (S - 1).bit_length()
            int_min = np.int32(-2 ** 31)
            r_all = _rb(r_s[...].reshape(N_BLK * 8, LANES))
            r_all = jnp.where(r_all == 0.0, 0.0, r_all)
            bits = lax.bitcast_convert_type(r_all, I32) >> 16
            code = jnp.where(bits < 0, bits ^ 0x7FFF, bits)
            code = jnp.where(r_all != r_all, -32768, code)
            row = lax.broadcasted_iota(I32, r_all.shape, 0)
            col = lax.broadcasted_iota(I32, r_all.shape, 1)
            tok = (row >> 3) * rows_blk + col * 8 + (row & 7)
            keys = jnp.where(col < rows_blk // 8, (code << idx_bits) | (S - 1 - tok), int_min)
            row_c = lax.broadcasted_iota(I32, (TOP_C, LANES), 0)
            best_keys = jnp.zeros((TOP_C, LANES), I32)
            for c in range(TOP_C):
                best = jnp.max(jnp.max(keys, axis=0, keepdims=True), axis=1, keepdims=True)
                best_keys = jnp.where(row_c == c, best, best_keys)
                keys = jnp.where(keys == best, int_min, keys)
            best_code = best_keys >> idx_bits
            st["r"] = lax.bitcast_convert_type(
                jnp.where(best_code < 0, best_code ^ 0x7FFF, best_code) << 16, F32)
            best_tok = S - 1 - (best_keys & (2 ** idx_bits - 1))
            st["idx"] = [jnp.max(jnp.where(row_c == c, best_tok, 0)) for c in range(TOP_C)]

        def gather():
            st["x"] = jnp.concatenate([act_load(XN, t, 1) for t in st["idx"]], axis=0)
            st["h"] = []

        def hidden(f0, f1):
            gate = _rb(_dot(st["x"], wg_s[f0:f1, :], _NT))
            up = _rb(_dot(st["x"], wu_s[f0:f1, :], _NT))
            st["h"].append(_silu(gate) * up)

        def down():
            st["y"] = _dot(jnp.concatenate(st["h"], axis=1), wd_s[...])

        def scatter():
            y = _rb(st["y"]) * _sigmoid(st["r"][:, :1])
            gate = _silu(st["x"] + (st["x"] * 0.0 + y))
            for c, t in enumerate(st["idx"]):
                act_store(GATE, t, gate[c:c + 1])

        n_f = wg_s.shape[0]
        nothing = lambda: None
        return ([select] + [nothing] * FFN_W0 + [gather]
                + [functools.partial(hidden, f, min(f + FFN_COLS, n_f)) for f in range(0, n_f, FFN_COLS)]
                + [nothing, down, nothing, scatter])

    def norm_early(i, carry):
        n = n_seg // LNPRE_IT
        xp = xp_s[pl.ds(i * n, n)].astype(F32).reshape(n * PRE_ROWS, D)
        rows = pl.ds(pl.multiple_of(i * n * PRE_ROWS, n * PRE_ROWS), n * PRE_ROWS)
        xpre_s[rows, :] = _layernorm(xp).astype(BF16)
        return carry

    with jax.named_scope("lnpre"):
        xp_copy.wait()
        lax.fori_loop(0, LNPRE_IT, norm_early, 0)

    with jax.named_scope("first"):
        p = 0
        for i, n in enumerate(FIRST):
            pairs_wait(p, n, SEM_FIRST + i)
            project_early(p, n, [])
            p += n

    def pre_block(it, carry):
        p_first = sum(FIRST) + it * pair_blk
        pairs_wait(p_first, pair_blk, SEM_BLK + it)
        x_copy(it, 1, SEM_BLK + it).wait()
        project_early(p_first, pair_blk, norm_work(it))
        return carry

    with jax.named_scope("pre"):
        lax.fori_loop(0, N_BLK, pre_block, 0)

    with jax.named_scope("last"):
        pairs_wait(n_pair - LAST, LAST, SEM_LAST)
        for cp in ffn_copies:
            cp.wait()
        project_early(n_pair - LAST, LAST, routed_ffn_work())
    with jax.named_scope("wowait"):
        for cp in wo_copies:
            cp.wait()

    hpg = LANES // L
    groups = [list(range(h, min(h + hpg, H))) for h in range(0, H, hpg)]
    lane = lax.broadcasted_iota(I32, (L, LANES), 1)
    key_j = lax.broadcasted_iota(I32, (L, LANES), 0)
    qry_t = lane
    for i in range(1, hpg):
        qry_t = jnp.where(lane >= i * L, lane - i * L, qry_t)
    allowed = (qry_t >= seg) | (key_j >= seg) | (key_j <= qry_t)

    def step(s, mem):
        r0 = pl.multiple_of(s * seg, seg)
        p0 = pl.multiple_of(s * PRE_ROWS, PRE_ROWS)
        h_rest = jnp.concatenate(
            [act_load(XN + PRE_ROWS, r0, seg - PRE_ROWS), mem], axis=0).astype(BF16)

        def project(m, heads, k0=0, k1=D):
            w = jnp.concatenate(
                [pltpu.bitcast(w_s[m * H + h, k0 // 2:k1 // 2, :], BF16) for h in heads], axis=1)
            return _dot(h_rest[:, k0:k1], w)

        def with_early(m, heads, res):
            return [jnp.concatenate([act_s[pl.ds(PRE + (m * H + h) * n_pre + p0, PRE_ROWS), :],
                                     res[:, j * E:(j + 1) * E]], axis=0)
                    for j, h in enumerate(heads)]

        def scores(q, k):
            n = len(q)
            qs = jnp.concatenate(q + [jnp.zeros((LANES - n * L, E), F32)], axis=0).astype(BF16)
            st = _dot(jnp.concatenate(k, axis=0), qs, _NT)
            merged = st[:L]
            for i in range(1, n):
                merged = jnp.where(lane >= i * L, st[i * L:(i + 1) * L], merged)
            sc = jnp.where(allowed, merged * scale, -1e9)
            e = jnp.exp(sc - jnp.max(sc, axis=0, keepdims=True))
            return e / jnp.sum(e, axis=0, keepdims=True)

        def mix(pt, v):
            p = jnp.concatenate([pt, jnp.zeros((LANES - L, LANES), F32)], axis=0).T
            outs = []
            for i, vh in enumerate(v):
                vp = jnp.concatenate([vh, jnp.zeros((LANES - L, E), F32)], axis=0).astype(BF16)
                outs.append(_dot(p[i * L:(i + 1) * L], vp))
            return outs

        n_g = len(groups)
        wo32 = wo_s.bitcast(U32)

        def out_proj(n, outs, h0):
            lhs = jnp.concatenate(
                [jnp.concatenate([oh[seg:], oh[:seg]], axis=0) for oh in outs], axis=1)
            rows = slice(h0 * E // 2, (h0 + len(outs)) * E // 2)
            return _dot(lhs, pltpu.bitcast(wo32[n, rows, :], BF16))

        q, k, v, probs, o = {}, {}, {}, {}, {}
        k_split = D - LANES
        head_start = {(m, g): project(m, groups[g], 0, k_split)
                      for g in range(N_SPLIT) for m in range(2)}
        for t in range(2 * n_g):
            if t < n_g:
                for m, dst in ((0, q), (1, k)):
                    if (m, t) in head_start:
                        res = project(m, groups[t], k_split, D) + head_start[m, t]
                    else:
                        res = project(m, groups[t])
                    dst[t] = with_early(m, groups[t], res)
            else:
                v[t - n_g] = with_early(2, groups[t - n_g], project(2, groups[t - n_g]))
            gs = t - LAG_S
            if 0 <= gs < n_g:
                probs[gs] = scores(q[gs], k[gs])
            gp = t - n_g - LAG_P
            if 0 <= gp < n_g:
                o[gp] = mix(probs[gp], v[gp])
        n_early = n_g - LAG_P
        early = [oh for g in range(n_early) for oh in o[g]]
        col0 = None
        cuts = [len(early) * i // LAG_P for i in range(LAG_P + 1)]
        for i in range(LAG_P):
            part = out_proj(0, early[cuts[i]:cuts[i + 1]], cuts[i])
            col0 = part if col0 is None else part + col0
            o[n_early + i] = mix(probs[n_early + i], v[n_early + i])
        late = [oh for g in range(n_early, n_g) for oh in o[g]]
        cols = [None] + [out_proj(1, early + late, 0)]
        cols[0] = out_proj(0, late, len(early)) + col0
        cols += [out_proj(n, early + late, 0) for n in range(2, n_col)]
        res = jnp.concatenate(cols, axis=1)
        out = x_s[s].astype(F32) + res[M:] * act_load(GATE, r0, seg)
        out_s[s] = out.astype(BF16)
        pltpu.make_async_copy(out_s.at[s], out_hbm.at[s], sem_out).start()
        return res[:M]

    with jax.named_scope("main"):
        lax.fori_loop(0, DBG_STEPS, step, mem0_ref[...].astype(F32), unroll=UNROLL)
    done = out_s.at[pl.ds(0, DBG_STEPS)]
    pltpu.make_async_copy(done, done, sem_out).wait()


@functools.partial(jax.jit, static_argnames=("A_seg_len",))
def pallas_recurrent_scan__memory_aug_recurrent_mem_tr__moe_arch_mod__prompt_kernel(
    A_x: jax.Array,
    A_mem0: jax.Array,
    A_Wq: jax.Array,
    A_Wk: jax.Array,
    A_Wv: jax.Array,
    A_Wo: jax.Array,
    A_seg_len: int,
    B_x: jax.Array,
    B_w_r: jax.Array,
    B_w_gate: jax.Array,
    B_w_up: jax.Array,
    B_w_down: jax.Array,
):
    del B_x
    B, S, D = A_x.shape
    _, H, E = A_Wq.shape
    M = A_mem0.shape[1]
    Fh = B_w_gate.shape[1]
    seg = int(A_seg_len)
    n_seg = S // seg

    hbm = pl.BlockSpec(memory_space=pltpu.HBM)
    vmem = pl.BlockSpec(memory_space=pltpu.VMEM)
    out = pl.pallas_call(
        _kernel,
        out_shape=jax.ShapeDtypeStruct((n_seg, seg, D), A_x.dtype),
        in_specs=[hbm, vmem, hbm, hbm, hbm, hbm, vmem, hbm, hbm, hbm],
        out_specs=hbm,
        scratch_shapes=[
            pltpu.VMEM((n_seg, seg, D), BF16),
            pltpu.VMEM((n_seg, PRE_ROWS, D), BF16),
            pltpu.VMEM((n_seg * PRE_ROWS, D), BF16),
            pltpu.VMEM((3 * H // 2, D, E), U32),
            pltpu.VMEM((3 * H, D // 2, E), U32),
            pltpu.VMEM((D // LANES, H * E, LANES), BF16),
            pltpu.VMEM((Fh, D), BF16),
            pltpu.VMEM((Fh, D), BF16),
            pltpu.VMEM((Fh, D), BF16),
            pltpu.VMEM((2 * (D // LANES) * S + 3 * H * n_seg * PRE_ROWS, LANES), F32),
            pltpu.VMEM((N_BLK, 8, LANES), F32),
            pltpu.VMEM((n_seg, seg, D), BF16),
            pltpu.SemaphoreType.DMA((N_BLK + 3 + len(FIRST),)),
            pltpu.SemaphoreType.DMA(()),
        ],
        compiler_params=pltpu.CompilerParams(vmem_limit_bytes=110 * 1024 * 1024),
    )(A_x.reshape(n_seg, seg, D), A_mem0.reshape(M, D), A_Wq, A_Wk, A_Wv, A_Wo.reshape(H * E, D),
      B_w_r, B_w_gate.T, B_w_up.T, B_w_down)
    return out.reshape(B, S, D)
```

```python
import functools

import jax
import jax.numpy as jnp
import numpy as np
from jax import lax
import jax.experimental.pallas as pl
import jax.experimental.pallas.tpu as pltpu

F32 = jnp.float32
BF16 = jnp.bfloat16
U32 = jnp.uint32
I32 = jnp.int32

TOP_C = 8
EPS_BF16 = 1.0013580322265625e-05
LANES = 128
SUBLANES = 8

EARLY_ROWS = 8
EARLY_PARTS = 2
EARLY_M = 64
FIRST_PAIRS = 4
LAST_PAIRS = 4
N_BLK = 8
FFN_COLS = 256
LAG_SCORES = 3
LAG_MIX = 3
UNROLL = 8

_NN = (((1,), (0,)), ((), ()))
_NT = (((1,), (1,)), ((), ()))


def _rb(x):
    return x.astype(BF16).astype(F32)


def _dot(a, b, dims=_NN):
    return lax.dot_general(a, b, dims, preferred_element_type=F32)


def _aligned(i, n):
    return i if isinstance(i, int) else pl.multiple_of(i, n)


def _layernorm(x):
    inv_n = 1.0 / x.shape[-1]
    mean = jnp.sum(x, axis=-1, keepdims=True) * inv_n
    c = x - mean
    var = jnp.sum(c * c, axis=-1, keepdims=True) * inv_n
    sd = _rb(jnp.sqrt(_rb(_rb(var) + EPS_BF16)))
    return _rb(_rb(x - _rb(mean)) * (1.0 / sd))


def _sigmoid(x):
    return 1.0 / (1.0 + jnp.exp(-x))


def _silu(x):
    return x * _sigmoid(x)


def _kernel(x_hbm, mem0_ref, wq_hbm, wk_hbm, wv_hbm, wo_hbm, wr_ref, wg_hbm, wu_hbm, wd_hbm,
            out_hbm,
            x_s, xe_s, xen_s, raw_s, w_s, wo_s, wg_s, wu_s, wd_s, act_s, r_s, out_s,
            sem, sem_out):
    n_seg, seg, D = x_hbm.shape
    S = n_seg * seg
    H, E = wq_hbm.shape[1], wq_hbm.shape[2]
    M = mem0_ref.shape[0]
    L = seg + M
    n_col = D // LANES
    n_pair = 3 * H // 2
    n_early = n_seg * EARLY_ROWS
    seg_blk = n_seg // N_BLK
    rows_blk = seg_blk * seg
    pair_blk = (n_pair - FIRST_PAIRS - LAST_PAIRS) // N_BLK
    assert FIRST_PAIRS + N_BLK * pair_blk + LAST_PAIRS == n_pair
    assert rows_blk // SUBLANES <= LANES

    XN, GATE, EARLY = 0, n_col * S, 2 * n_col * S

    def act_load(base, r, n):
        return jnp.concatenate([act_s[pl.ds(base + c * S + r, n), :] for c in range(n_col)],
                               axis=1)

    def act_store(base, r, val, stride=S):
        for c in range(val.shape[1] // LANES):
            act_s[pl.ds(base + c * stride + r, val.shape[0]), :] = val[:, c * LANES:(c + 1) * LANES]

    SEM_EARLY, SEM_FIRST = 0, EARLY_PARTS
    SEM_BLK = SEM_FIRST + FIRST_PAIRS
    SEM_LAST, SEM_WO = SEM_BLK + N_BLK, SEM_BLK + N_BLK + 1

    seg_part = n_seg // EARLY_PARTS
    early_copies = [
        pltpu.make_async_copy(x_hbm.at[pl.ds(i * seg_part, seg_part), pl.ds(0, EARLY_ROWS), :],
                              xe_s.at[pl.ds(i * seg_part, seg_part)], sem.at[SEM_EARLY + i])
        for i in range(EARLY_PARTS)]
    ffn_copies = [pltpu.make_async_copy(src, dst, sem.at[SEM_LAST])
                  for src, dst in ((wg_hbm, wg_s), (wu_hbm, wu_s), (wd_hbm, wd_s))]
    wo_copies = [pltpu.make_async_copy(wo_hbm.at[:, pl.ds(n * LANES, LANES)], wo_s.at[n],
                                       sem.at[SEM_WO]) for n in range(n_col)]

    def x_copy(i):
        blk = pl.ds(i * seg_blk, seg_blk)
        return pltpu.make_async_copy(x_hbm.at[blk], x_s.at[blk], sem.at[SEM_BLK + i])

    def pairs_start(p0, n, sem_id):
        for p in range(p0, p0 + n):
            m, c = divmod(p, H // 2)
            src = (wq_hbm, wk_hbm, wv_hbm)[m].bitcast(U32).at[:, c, :]
            pltpu.make_async_copy(src, raw_s.at[p], sem.at[sem_id]).start()

    def pairs_wait(p0, n, sem_id):
        dst = raw_s.at[pl.ds(p0, n)]
        pltpu.make_async_copy(dst, dst, sem.at[sem_id]).wait()

    for cp in early_copies:
        cp.start()
    for p in range(FIRST_PAIRS):
        pairs_start(p, 1, SEM_FIRST + p)
    for i in range(N_BLK):
        pairs_start(FIRST_PAIRS + i * pair_blk, pair_blk, SEM_BLK + i)
        x_copy(i).start()
    pairs_start(n_pair - LAST_PAIRS, LAST_PAIRS, SEM_LAST)
    for cp in ffn_copies + wo_copies:
        cp.start()

    def project_early(p0, n, side_work):
        n_piece = n * (n_early // EARLY_M)
        piece = done = 0
        for j in range(n):
            p = p0 + j
            even = raw_s[p, pl.ds(0, D // 2, stride=2), :]
            odd = raw_s[p, pl.ds(1, D // 2, stride=2), :]
            lo = (even & np.uint32(0xFFFF)) | (odd << 16)
            hi = (even >> 16) | (odd & np.uint32(0xFFFF0000))
            w_s[2 * p] = lo
            w_s[2 * p + 1] = hi
            w = jnp.concatenate([pltpu.bitcast(lo, BF16), pltpu.bitcast(hi, BF16)], axis=1)
            for r in range(0, n_early, EARLY_M):
                res = _dot(xen_s[r:r + EARLY_M, :], w)
                act_store(EARLY, _aligned(2 * p * n_early + r, EARLY_M), res, n_early)
                piece += 1
                while done < min(len(side_work), -(-piece * len(side_work) // (n_piece - 2))):
                    side_work[done]()
                    done += 1

    wr = wr_ref[...].astype(F32).reshape(1, D)
    lane8 = lax.broadcasted_iota(I32, (SUBLANES, LANES), 1)

    def norm_work(blk):
        scores = [jnp.zeros((SUBLANES, LANES), F32)]
        n = rows_blk // SUBLANES

        def piece(i):
            sg, off = divmod(i * SUBLANES, seg)
            xn = _layernorm(x_s[blk * seg_blk + sg, off:off + SUBLANES, :].astype(F32))
            r0 = _aligned(blk * rows_blk + i * SUBLANES, SUBLANES)
            act_store(XN, r0, xn)
            act_store(GATE, r0, _silu(xn + xn * 0.0))
            scores[0] = jnp.where(lane8 == i, jnp.sum(xn * wr, axis=-1, keepdims=True), scores[0])
            if i == n - 1:
                r_s[blk] = scores[0]

        return [functools.partial(piece, i) for i in range(n)]

    def routed_ffn_work():
        st = {}

        def select():
            idx_bits = (S - 1).bit_length()
            int_min = np.int32(-2 ** 31)
            r_all = _rb(r_s[...].reshape(N_BLK * SUBLANES, LANES))
            r_all = jnp.where(r_all == 0.0, 0.0, r_all)
            bits = lax.bitcast_convert_type(r_all, I32) >> 16
            code = jnp.where(bits < 0, bits ^ 0x7FFF, bits)
            code = jnp.where(r_all != r_all, -32768, code)
            row = lax.broadcasted_iota(I32, r_all.shape, 0)
            col = lax.broadcasted_iota(I32, r_all.shape, 1)
            tok = (row >> 3) * rows_blk + col * SUBLANES + (row & 7)
            keys = jnp.where(col < rows_blk // SUBLANES, (code << idx_bits) | (S - 1 - tok),
                             int_min)
            row_c = lax.broadcasted_iota(I32, (TOP_C, LANES), 0)
            best_keys = jnp.zeros((TOP_C, LANES), I32)
            for c in range(TOP_C):
                best = jnp.max(jnp.max(keys, axis=0, keepdims=True), axis=1, keepdims=True)
                best_keys = jnp.where(row_c == c, best, best_keys)
                keys = jnp.where(keys == best, int_min, keys)
            best_code = best_keys >> idx_bits
            st["score"] = lax.bitcast_convert_type(
                jnp.where(best_code < 0, best_code ^ 0x7FFF, best_code) << 16, F32)
            best_tok = S - 1 - (best_keys & (2 ** idx_bits - 1))
            st["idx"] = [jnp.max(jnp.where(row_c == c, best_tok, 0)) for c in range(TOP_C)]

        def gather():
            st["x"] = jnp.concatenate([act_load(XN, t, 1) for t in st["idx"]], axis=0)
            st["h"] = []

        def hidden(f0, f1):
            gate = _rb(_dot(st["x"], wg_s[f0:f1, :], _NT))
            up = _rb(_dot(st["x"], wu_s[f0:f1, :], _NT))
            st["h"].append(_silu(gate) * up)

        def down():
            st["y"] = _dot(jnp.concatenate(st["h"], axis=1), wd_s[...])

        def scatter():
            y = _rb(st["y"]) * _sigmoid(st["score"][:, :1])
            gate = _silu(st["x"] + (st["x"] * 0.0 + y))
            for c, t in enumerate(st["idx"]):
                act_store(GATE, t, gate[c:c + 1])

        def pause():
            pass

        n_f = wg_s.shape[0]
        return ([select] + [pause] * 8 + [gather]
                + [functools.partial(hidden, f, min(f + FFN_COLS, n_f))
                   for f in range(0, n_f, FFN_COLS)]
                + [pause, down, pause, scatter])

    for i, cp in enumerate(early_copies):
        cp.wait()
        n = seg_part * EARLY_ROWS
        xe = xe_s[i * seg_part:(i + 1) * seg_part].astype(F32).reshape(n, D)
        xen_s[i * n:(i + 1) * n, :] = _layernorm(xe).astype(BF16)

    def first_pair(p, carry):
        pairs_wait(p, 1, SEM_FIRST + p)
        project_early(p, 1, [])
        return carry

    lax.fori_loop(0, FIRST_PAIRS, first_pair, 0)

    def middle_block(i, carry):
        p0 = FIRST_PAIRS + i * pair_blk
        pairs_wait(p0, pair_blk, SEM_BLK + i)
        x_copy(i).wait()
        project_early(p0, pair_blk, norm_work(i))
        return carry

    lax.fori_loop(0, N_BLK, middle_block, 0)

    pairs_wait(n_pair - LAST_PAIRS, LAST_PAIRS, SEM_LAST)
    for cp in ffn_copies:
        cp.wait()
    project_early(n_pair - LAST_PAIRS, LAST_PAIRS, routed_ffn_work())
    for cp in wo_copies:
        cp.wait()

    scale = E ** -0.5
    per_tile = LANES // L
    groups = [list(range(h, min(h + per_tile, H))) for h in range(0, H, per_tile)]
    n_g = len(groups)
    lane = lax.broadcasted_iota(I32, (L, LANES), 1)
    key_j = lax.broadcasted_iota(I32, (L, LANES), 0)
    qry_t = lane
    for i in range(1, per_tile):
        qry_t = jnp.where(lane >= i * L, lane - i * L, qry_t)
    allowed = (qry_t >= seg) | (key_j >= seg) | (key_j <= qry_t)
    wo_words = wo_s.bitcast(U32)

    def probabilities(q, k):
        n = len(q)
        qs = jnp.concatenate(q + [jnp.zeros((LANES - n * L, E), F32)], axis=0).astype(BF16)
        st = _dot(jnp.concatenate(k, axis=0), qs, _NT)
        merged = st[:L]
        for i in range(1, n):
            merged = jnp.where(lane >= i * L, st[i * L:(i + 1) * L], merged)
        sc = jnp.where(allowed, merged * scale, -1e9)
        e = jnp.exp(sc - jnp.max(sc, axis=0, keepdims=True))
        return e / jnp.sum(e, axis=0, keepdims=True)

    def mix(pt, v):
        p = jnp.concatenate([pt, jnp.zeros((LANES - L, LANES), F32)], axis=0).T
        outs = []
        for i, vh in enumerate(v):
            vp = jnp.concatenate([vh, jnp.zeros((LANES - L, E), F32)], axis=0).astype(BF16)
            o = _dot(p[i * L:(i + 1) * L], vp)
            outs.append(jnp.concatenate([o[seg:], o[:seg]], axis=0))
        return outs

    def out_proj(n, outs, h0):
        rows = slice(h0 * E // 2, (h0 + len(outs)) * E // 2)
        return _dot(jnp.concatenate(outs, axis=1), pltpu.bitcast(wo_words[n, rows, :], BF16))

    def step(s, mem):
        r0 = pl.multiple_of(s * seg, seg)
        e0 = pl.multiple_of(s * EARLY_ROWS, EARLY_ROWS)
        h = jnp.concatenate([act_load(XN + EARLY_ROWS, r0, seg - EARLY_ROWS), mem],
                            axis=0).astype(BF16)

        def project(m, heads, k0=0, k1=D):
            w = jnp.concatenate(
                [pltpu.bitcast(w_s[m * H + hd, k0 // 2:k1 // 2, :], BF16) for hd in heads], axis=1)
            return _dot(h[:, k0:k1], w)

        def with_early(m, heads, res):
            return [jnp.concatenate(
                [act_s[pl.ds(EARLY + (m * H + hd) * n_early + e0, EARLY_ROWS), :],
                 res[:, j * E:(j + 1) * E]], axis=0) for j, hd in enumerate(heads)]

        k_split = D - LANES
        head_start = [project(m, groups[0], 0, k_split) for m in range(2)]
        q, k, v, probs, o = {}, {}, {}, {}, {}
        for t in range(2 * n_g):
            if t < n_g:
                for m, dst in enumerate((q, k)):
                    if t == 0:
                        res = project(m, groups[t], k_split, D) + head_start[m]
                    else:
                        res = project(m, groups[t])
                    dst[t] = with_early(m, groups[t], res)
            else:
                v[t - n_g] = with_early(2, groups[t - n_g], project(2, groups[t - n_g]))
            g = t - LAG_SCORES
            if 0 <= g < n_g:
                probs[g] = probabilities(q[g], k[g])
            g = t - n_g - LAG_MIX
            if 0 <= g < n_g:
                o[g] = mix(probs[g], v[g])

        n_done = n_g - LAG_MIX
        ready = [oh for g in range(n_done) for oh in o[g]]
        cuts = [len(ready) * i // LAG_MIX for i in range(LAG_MIX + 1)]
        col0, late = None, []
        for i in range(LAG_MIX):
            part = out_proj(0, ready[cuts[i]:cuts[i + 1]], cuts[i])
            col0 = part if col0 is None else part + col0
            late += mix(probs[n_done + i], v[n_done + i])
        col1 = out_proj(1, ready + late, 0)
        col0 = out_proj(0, late, len(ready)) + col0
        res = jnp.concatenate(
            [col0, col1] + [out_proj(n, ready + late, 0) for n in range(2, n_col)], axis=1)

        out_s[s] = (x_s[s].astype(F32) + res[M:] * act_load(GATE, r0, seg)).astype(BF16)
        pltpu.make_async_copy(out_s.at[s], out_hbm.at[s], sem_out).start()
        return res[:M]

    lax.fori_loop(0, n_seg, step, mem0_ref[...].astype(F32), unroll=UNROLL)
    pltpu.make_async_copy(out_s, out_s, sem_out).wait()


@functools.partial(jax.jit, static_argnames=("A_seg_len",))
def pallas_recurrent_scan__memory_aug_recurrent_mem_tr__moe_arch_mod__prompt_kernel(
    A_x: jax.Array,
    A_mem0: jax.Array,
    A_Wq: jax.Array,
    A_Wk: jax.Array,
    A_Wv: jax.Array,
    A_Wo: jax.Array,
    A_seg_len: int,
    B_x: jax.Array,
    B_w_r: jax.Array,
    B_w_gate: jax.Array,
    B_w_up: jax.Array,
    B_w_down: jax.Array,
):
    del B_x
    B, S, D = A_x.shape
    _, H, E = A_Wq.shape
    M = A_mem0.shape[1]
    F = B_w_gate.shape[1]
    seg = int(A_seg_len)
    n_seg = S // seg
    n_col = D // LANES
    assert B == 1 and E == LANES and D % LANES == 0 and S == n_seg * seg

    hbm = pl.BlockSpec(memory_space=pltpu.HBM)
    vmem = pl.BlockSpec(memory_space=pltpu.VMEM)
    out = pl.pallas_call(
        _kernel,
        out_shape=jax.ShapeDtypeStruct((n_seg, seg, D), A_x.dtype),
        in_specs=[hbm, vmem, hbm, hbm, hbm, hbm, vmem, hbm, hbm, hbm],
        out_specs=hbm,
        scratch_shapes=[
            pltpu.VMEM((n_seg, seg, D), BF16),
            pltpu.VMEM((n_seg, EARLY_ROWS, D), BF16),
            pltpu.VMEM((n_seg * EARLY_ROWS, D), BF16),
            pltpu.VMEM((3 * H // 2, D, E), U32),
            pltpu.VMEM((3 * H, D // 2, E), U32),
            pltpu.VMEM((n_col, H * E, LANES), BF16),
            pltpu.VMEM((F, D), BF16),
            pltpu.VMEM((F, D), BF16),
            pltpu.VMEM((F, D), BF16),
            pltpu.VMEM((2 * n_col * S + 3 * H * n_seg * EARLY_ROWS, LANES), F32),
            pltpu.VMEM((N_BLK, SUBLANES, LANES), F32),
            pltpu.VMEM((n_seg, seg, D), BF16),
            pltpu.SemaphoreType.DMA((EARLY_PARTS + FIRST_PAIRS + N_BLK + 2,)),
            pltpu.SemaphoreType.DMA(()),
        ],
        compiler_params=pltpu.CompilerParams(vmem_limit_bytes=110 * 1024 * 1024),
    )(A_x.reshape(n_seg, seg, D), A_mem0.reshape(M, D), A_Wq, A_Wk, A_Wv, A_Wo.reshape(H * E, D),
      B_w_r, B_w_gate.T, B_w_up.T, B_w_down)
    return out.reshape(B, S, D)
```

```python
import functools

import jax
import jax.numpy as jnp
import numpy as np
from jax import lax
import jax.experimental.pallas as pl
import jax.experimental.pallas.tpu as pltpu

F32 = jnp.float32
BF16 = jnp.bfloat16
U32 = jnp.uint32
I32 = jnp.int32

TOP_C = 8
EPS_BF16 = 1.0013580322265625e-05
LANES = 128
SUBLANES = 8

EARLY_ROWS = 8
EARLY_PARTS = 2
EARLY_M = 64
FIRST_PAIRS = 4
LAST_PAIRS = 4
N_BLK = 8
FFN_COLS = 256
LAG_SCORES = 3
LAG_MIX = 3
UNROLL = 8

_NN = (((1,), (0,)), ((), ()))
_NT = (((1,), (1,)), ((), ()))


def _rb(x):
    return x.astype(BF16).astype(F32)


def _dot(a, b, dims=_NN):
    return lax.dot_general(a, b, dims, preferred_element_type=F32)


def _aligned(i, n):
    return i if isinstance(i, int) else pl.multiple_of(i, n)


def _layernorm(x):
    inv_n = 1.0 / x.shape[-1]
    mean = jnp.sum(x, axis=-1, keepdims=True) * inv_n
    c = x - mean
    var = jnp.sum(c * c, axis=-1, keepdims=True) * inv_n
    sd = _rb(jnp.sqrt(_rb(_rb(var) + EPS_BF16)))
    return _rb(_rb(x - _rb(mean)) * (1.0 / sd))


def _sigmoid(x):
    return 1.0 / (1.0 + jnp.exp(-x))


def _silu(x):
    return x * _sigmoid(x)


def _kernel(x_hbm, mem0_hbm, wq_hbm, wk_hbm, wv_hbm, wo_hbm, wr_hbm, wg_hbm, wu_hbm, wd_hbm,
            out_hbm,
            x_s, xe_s, xen_s, raw_s, w_s, wo_s, wg_s, wu_s, wd_s, act_s, r_s, out_s, mem0_s, wr_s,
            sem, sem_out):
    n_seg, seg, D = x_hbm.shape
    S = n_seg * seg
    H, E = wq_hbm.shape[1], wq_hbm.shape[2]
    M = mem0_hbm.shape[0]
    L = seg + M
    n_col = D // LANES
    n_pair = 3 * H // 2
    n_early = n_seg * EARLY_ROWS
    seg_blk = n_seg // N_BLK
    rows_blk = seg_blk * seg
    pair_blk = (n_pair - FIRST_PAIRS - LAST_PAIRS) // N_BLK
    assert FIRST_PAIRS + N_BLK * pair_blk + LAST_PAIRS == n_pair
    assert rows_blk // SUBLANES <= LANES

    XN, GATE, EARLY = 0, n_col * S, 2 * n_col * S

    def act_load(base, r, n):
        return jnp.concatenate([act_s[pl.ds(base + c * S + r, n), :] for c in range(n_col)],
                               axis=1)

    def act_store(base, r, val, stride=S):
        for c in range(val.shape[1] // LANES):
            act_s[pl.ds(base + c * stride + r, val.shape[0]), :] = val[:, c * LANES:(c + 1) * LANES]

    SEM_EARLY, SEM_FIRST = 0, EARLY_PARTS
    SEM_BLK = SEM_FIRST + FIRST_PAIRS
    SEM_SMALL, SEM_LAST, SEM_WO = (SEM_BLK + N_BLK + i for i in range(3))

    seg_part = n_seg // EARLY_PARTS
    early_copies = [
        pltpu.make_async_copy(x_hbm.at[pl.ds(i * seg_part, seg_part), pl.ds(0, EARLY_ROWS), :],
                              xe_s.at[pl.ds(i * seg_part, seg_part)], sem.at[SEM_EARLY + i])
        for i in range(EARLY_PARTS)]
    small_copies = [pltpu.make_async_copy(src, dst, sem.at[SEM_SMALL])
                    for src, dst in ((wr_hbm, wr_s), (mem0_hbm, mem0_s))]
    ffn_copies = [pltpu.make_async_copy(src, dst, sem.at[SEM_LAST])
                  for src, dst in ((wg_hbm, wg_s), (wu_hbm, wu_s), (wd_hbm, wd_s))]
    wo_copies = [pltpu.make_async_copy(wo_hbm.at[:, pl.ds(n * LANES, LANES)], wo_s.at[n],
                                       sem.at[SEM_WO]) for n in range(n_col)]

    def x_copy(i):
        blk = pl.ds(i * seg_blk, seg_blk)
        return pltpu.make_async_copy(x_hbm.at[blk], x_s.at[blk], sem.at[SEM_BLK + i])

    def pairs_start(p0, n, sem_id):
        for p in range(p0, p0 + n):
            m, c = divmod(p, H // 2)
            src = (wq_hbm, wk_hbm, wv_hbm)[m].bitcast(U32).at[:, c, :]
            pltpu.make_async_copy(src, raw_s.at[p], sem.at[sem_id]).start()

    def pairs_wait(p0, n, sem_id):
        dst = raw_s.at[pl.ds(p0, n)]
        pltpu.make_async_copy(dst, dst, sem.at[sem_id]).wait()

    for cp in early_copies:
        cp.start()
    for p in range(FIRST_PAIRS):
        pairs_start(p, 1, SEM_FIRST + p)
    for cp in small_copies:
        cp.start()
    for i in range(N_BLK):
        pairs_start(FIRST_PAIRS + i * pair_blk, pair_blk, SEM_BLK + i)
        x_copy(i).start()
    pairs_start(n_pair - LAST_PAIRS, LAST_PAIRS, SEM_LAST)
    for cp in ffn_copies + wo_copies:
        cp.start()

    def project_early(p0, n, side_work):
        n_piece = n * (n_early // EARLY_M)
        piece = done = 0
        for j in range(n):
            p = p0 + j
            even = raw_s[p, pl.ds(0, D // 2, stride=2), :]
            odd = raw_s[p, pl.ds(1, D // 2, stride=2), :]
            lo = (even & np.uint32(0xFFFF)) | (odd << 16)
            hi = (even >> 16) | (odd & np.uint32(0xFFFF0000))
            w_s[2 * p] = lo
            w_s[2 * p + 1] = hi
            w = jnp.concatenate([pltpu.bitcast(lo, BF16), pltpu.bitcast(hi, BF16)], axis=1)
            for r in range(0, n_early, EARLY_M):
                res = _dot(xen_s[r:r + EARLY_M, :], w)
                act_store(EARLY, _aligned(2 * p * n_early + r, EARLY_M), res, n_early)
                piece += 1
                while done < min(len(side_work), -(-piece * len(side_work) // (n_piece - 2))):
                    side_work[done]()
                    done += 1

    lane8 = lax.broadcasted_iota(I32, (SUBLANES, LANES), 1)

    def norm_work(blk, wr):
        scores = [jnp.zeros((SUBLANES, LANES), F32)]
        n = rows_blk // SUBLANES

        def piece(i):
            sg, off = divmod(i * SUBLANES, seg)
            xn = _layernorm(x_s[blk * seg_blk + sg, off:off + SUBLANES, :].astype(F32))
            r0 = _aligned(blk * rows_blk + i * SUBLANES, SUBLANES)
            act_store(XN, r0, xn)
            act_store(GATE, r0, _silu(xn + xn * 0.0))
            scores[0] = jnp.where(lane8 == i, jnp.sum(xn * wr, axis=-1, keepdims=True), scores[0])
            if i == n - 1:
                r_s[blk] = scores[0]

        return [functools.partial(piece, i) for i in range(n)]

    def routed_ffn_work():
        st = {}

        def select():
            idx_bits = (S - 1).bit_length()
            int_min = np.int32(-2 ** 31)
            r_all = _rb(r_s[...].reshape(N_BLK * SUBLANES, LANES))
            r_all = jnp.where(r_all == 0.0, 0.0, r_all)
            bits = lax.bitcast_convert_type(r_all, I32) >> 16
            code = jnp.where(bits < 0, bits ^ 0x7FFF, bits)
            code = jnp.where(r_all != r_all, -32768, code)
            row = lax.broadcasted_iota(I32, r_all.shape, 0)
            col = lax.broadcasted_iota(I32, r_all.shape, 1)
            tok = (row >> 3) * rows_blk + col * SUBLANES + (row & 7)
            keys = jnp.where(col < rows_blk // SUBLANES, (code << idx_bits) | (S - 1 - tok),
                             int_min)
            row_c = lax.broadcasted_iota(I32, (TOP_C, LANES), 0)
            best_keys = jnp.zeros((TOP_C, LANES), I32)
            for c in range(TOP_C):
                best = jnp.max(jnp.max(keys, axis=0, keepdims=True), axis=1, keepdims=True)
                best_keys = jnp.where(row_c == c, best, best_keys)
                keys = jnp.where(keys == best, int_min, keys)
            best_code = best_keys >> idx_bits
            st["score"] = lax.bitcast_convert_type(
                jnp.where(best_code < 0, best_code ^ 0x7FFF, best_code) << 16, F32)
            best_tok = S - 1 - (best_keys & (2 ** idx_bits - 1))
            st["idx"] = [jnp.max(jnp.where(row_c == c, best_tok, 0)) for c in range(TOP_C)]

        def gather():
            st["x"] = jnp.concatenate([act_load(XN, t, 1) for t in st["idx"]], axis=0)
            st["h"] = []

        def hidden(f0, f1):
            gate = _rb(_dot(st["x"], wg_s[f0:f1, :], _NT))
            up = _rb(_dot(st["x"], wu_s[f0:f1, :], _NT))
            st["h"].append(_silu(gate) * up)

        def down():
            st["y"] = _dot(jnp.concatenate(st["h"], axis=1), wd_s[...])

        def scatter():
            y = _rb(st["y"]) * _sigmoid(st["score"][:, :1])
            gate = _silu(st["x"] + (st["x"] * 0.0 + y))
            for c, t in enumerate(st["idx"]):
                act_store(GATE, t, gate[c:c + 1])

        def pause():
            pass

        n_f = wg_s.shape[0]
        return ([select] + [pause] * 8 + [gather]
                + [functools.partial(hidden, f, min(f + FFN_COLS, n_f))
                   for f in range(0, n_f, FFN_COLS)]
                + [pause, down, pause, scatter])

    for i, cp in enumerate(early_copies):
        cp.wait()
        n = seg_part * EARLY_ROWS
        xe = xe_s[i * seg_part:(i + 1) * seg_part].astype(F32).reshape(n, D)
        xen_s[i * n:(i + 1) * n, :] = _layernorm(xe).astype(BF16)

    def first_pair(p, carry):
        pairs_wait(p, 1, SEM_FIRST + p)
        project_early(p, 1, [])
        return carry

    lax.fori_loop(0, FIRST_PAIRS, first_pair, 0)

    for cp in small_copies:
        cp.wait()
    wr = wr_s[...].astype(F32).reshape(1, D)

    def middle_block(i, carry):
        p0 = FIRST_PAIRS + i * pair_blk
        pairs_wait(p0, pair_blk, SEM_BLK + i)
        x_copy(i).wait()
        project_early(p0, pair_blk, norm_work(i, wr))
        return carry

    lax.fori_loop(0, N_BLK, middle_block, 0)

    pairs_wait(n_pair - LAST_PAIRS, LAST_PAIRS, SEM_LAST)
    for cp in ffn_copies:
        cp.wait()
    project_early(n_pair - LAST_PAIRS, LAST_PAIRS, routed_ffn_work())
    for cp in wo_copies:
        cp.wait()

    scale = E ** -0.5
    per_tile = LANES // L
    groups = [list(range(h, min(h + per_tile, H))) for h in range(0, H, per_tile)]
    n_g = len(groups)
    lane = lax.broadcasted_iota(I32, (L, LANES), 1)
    key_j = lax.broadcasted_iota(I32, (L, LANES), 0)
    qry_t = lane
    for i in range(1, per_tile):
        qry_t = jnp.where(lane >= i * L, lane - i * L, qry_t)
    allowed = (qry_t >= seg) | (key_j >= seg) | (key_j <= qry_t)
    wo_words = wo_s.bitcast(U32)

    def probabilities(q, k):
        n = len(q)
        qs = jnp.concatenate(q + [jnp.zeros((LANES - n * L, E), F32)], axis=0).astype(BF16)
        st = _dot(jnp.concatenate(k, axis=0), qs, _NT)
        merged = st[:L]
        for i in range(1, n):
            merged = jnp.where(lane >= i * L, st[i * L:(i + 1) * L], merged)
        sc = jnp.where(allowed, merged * scale, -1e9)
        e = jnp.exp(sc - jnp.max(sc, axis=0, keepdims=True))
        return e / jnp.sum(e, axis=0, keepdims=True)

    def mix(pt, v):
        p = jnp.concatenate([pt, jnp.zeros((LANES - L, LANES), F32)], axis=0).T
        outs = []
        for i, vh in enumerate(v):
            vp = jnp.concatenate([vh, jnp.zeros((LANES - L, E), F32)], axis=0).astype(BF16)
            o = _dot(p[i * L:(i + 1) * L], vp)
            outs.append(jnp.concatenate([o[seg:], o[:seg]], axis=0))
        return outs

    def out_proj(n, outs, h0):
        rows = slice(h0 * E // 2, (h0 + len(outs)) * E // 2)
        return _dot(jnp.concatenate(outs, axis=1), pltpu.bitcast(wo_words[n, rows, :], BF16))

    def step(s, mem):
        r0 = pl.multiple_of(s * seg, seg)
        e0 = pl.multiple_of(s * EARLY_ROWS, EARLY_ROWS)
        h = jnp.concatenate([act_load(XN + EARLY_ROWS, r0, seg - EARLY_ROWS), mem],
                            axis=0).astype(BF16)

        def project(m, heads, k0=0, k1=D):
            w = jnp.concatenate(
                [pltpu.bitcast(w_s[m * H + hd, k0 // 2:k1 // 2, :], BF16) for hd in heads], axis=1)
            return _dot(h[:, k0:k1], w)

        def with_early(m, heads, res):
            return [jnp.concatenate(
                [act_s[pl.ds(EARLY + (m * H + hd) * n_early + e0, EARLY_ROWS), :],
                 res[:, j * E:(j + 1) * E]], axis=0) for j, hd in enumerate(heads)]

        k_split = D - LANES
        head_start = [project(m, groups[0], 0, k_split) for m in range(2)]
        q, k, v, probs, o = {}, {}, {}, {}, {}
        for t in range(2 * n_g):
            if t < n_g:
                for m, dst in enumerate((q, k)):
                    if t == 0:
                        res = project(m, groups[t], k_split, D) + head_start[m]
                    else:
                        res = project(m, groups[t])
                    dst[t] = with_early(m, groups[t], res)
            else:
                v[t - n_g] = with_early(2, groups[t - n_g], project(2, groups[t - n_g]))
            g = t - LAG_SCORES
            if 0 <= g < n_g:
                probs[g] = probabilities(q[g], k[g])
            g = t - n_g - LAG_MIX
            if 0 <= g < n_g:
                o[g] = mix(probs[g], v[g])

        n_done = n_g - LAG_MIX
        ready = [oh for g in range(n_done) for oh in o[g]]
        cuts = [len(ready) * i // LAG_MIX for i in range(LAG_MIX + 1)]
        col0, late = None, []
        for i in range(LAG_MIX):
            part = out_proj(0, ready[cuts[i]:cuts[i + 1]], cuts[i])
            col0 = part if col0 is None else part + col0
            late += mix(probs[n_done + i], v[n_done + i])
        col1 = out_proj(1, ready + late, 0)
        col0 = out_proj(0, late, len(ready)) + col0
        res = jnp.concatenate(
            [col0, col1] + [out_proj(n, ready + late, 0) for n in range(2, n_col)], axis=1)

        out_s[s] = (x_s[s].astype(F32) + res[M:] * act_load(GATE, r0, seg)).astype(BF16)
        pltpu.make_async_copy(out_s.at[s], out_hbm.at[s], sem_out).start()
        return res[:M]

    lax.fori_loop(0, n_seg, step, mem0_s[...].astype(F32), unroll=UNROLL)
    pltpu.make_async_copy(out_s, out_s, sem_out).wait()


@functools.partial(jax.jit, static_argnames=("A_seg_len",))
def pallas_recurrent_scan__memory_aug_recurrent_mem_tr__moe_arch_mod__prompt_kernel(
    A_x: jax.Array,
    A_mem0: jax.Array,
    A_Wq: jax.Array,
    A_Wk: jax.Array,
    A_Wv: jax.Array,
    A_Wo: jax.Array,
    A_seg_len: int,
    B_x: jax.Array,
    B_w_r: jax.Array,
    B_w_gate: jax.Array,
    B_w_up: jax.Array,
    B_w_down: jax.Array,
):
    del B_x
    B, S, D = A_x.shape
    _, H, E = A_Wq.shape
    M = A_mem0.shape[1]
    F = B_w_gate.shape[1]
    seg = int(A_seg_len)
    n_seg = S // seg
    n_col = D // LANES
    assert B == 1 and E == LANES and D % LANES == 0 and S == n_seg * seg

    hbm = pl.BlockSpec(memory_space=pltpu.HBM)
    out = pl.pallas_call(
        _kernel,
        out_shape=jax.ShapeDtypeStruct((n_seg, seg, D), A_x.dtype),
        in_specs=[hbm] * 10,
        out_specs=hbm,
        scratch_shapes=[
            pltpu.VMEM((n_seg, seg, D), BF16),
            pltpu.VMEM((n_seg, EARLY_ROWS, D), BF16),
            pltpu.VMEM((n_seg * EARLY_ROWS, D), BF16),
            pltpu.VMEM((3 * H // 2, D, E), U32),
            pltpu.VMEM((3 * H, D // 2, E), U32),
            pltpu.VMEM((n_col, H * E, LANES), BF16),
            pltpu.VMEM((F, D), BF16),
            pltpu.VMEM((F, D), BF16),
            pltpu.VMEM((F, D), BF16),
            pltpu.VMEM((2 * n_col * S + 3 * H * n_seg * EARLY_ROWS, LANES), F32),
            pltpu.VMEM((N_BLK, SUBLANES, LANES), F32),
            pltpu.VMEM((n_seg, seg, D), BF16),
            pltpu.VMEM((M, D), BF16),
            pltpu.VMEM((D,), BF16),
            pltpu.SemaphoreType.DMA((EARLY_PARTS + FIRST_PAIRS + N_BLK + 3,)),
            pltpu.SemaphoreType.DMA(()),
        ],
        compiler_params=pltpu.CompilerParams(vmem_limit_bytes=110 * 1024 * 1024),
    )(A_x.reshape(n_seg, seg, D), A_mem0.reshape(M, D), A_Wq, A_Wk, A_Wv, A_Wo.reshape(H * E, D),
      B_w_r, B_w_gate.T, B_w_up.T, B_w_down)
    return out.reshape(B, S, D)
```

```python
import functools

import jax
import jax.numpy as jnp
import numpy as np
from jax import lax
import jax.experimental.pallas as pl
import jax.experimental.pallas.tpu as pltpu

F32 = jnp.float32
BF16 = jnp.bfloat16
U32 = jnp.uint32
I32 = jnp.int32

TOP_C = 8
EPS_BF16 = 1.0013580322265625e-05
LANES = 128
SUBLANES = 8

EARLY_ROWS = 8
EARLY_PARTS = 2
EARLY_M = 64
FIRST_PAIRS = 4
LAST_PAIRS = 4
N_BLK = 8
FFN_COLS = 256
LAG_SCORES = 3
LAG_MIX = 3
UNROLL = 8

_NN = (((1,), (0,)), ((), ()))
_NT = (((1,), (1,)), ((), ()))


def _rb(x):
    return x.astype(BF16).astype(F32)


def _dot(a, b, dims=_NN):
    return lax.dot_general(a, b, dims, preferred_element_type=F32)


def _aligned(i, n):
    return i if isinstance(i, int) else pl.multiple_of(i, n)


def _layernorm(x):
    inv_n = 1.0 / x.shape[-1]
    mean = jnp.sum(x, axis=-1, keepdims=True) * inv_n
    c = x - mean
    var = jnp.sum(c * c, axis=-1, keepdims=True) * inv_n
    sd = _rb(jnp.sqrt(_rb(_rb(var) + EPS_BF16)))
    return _rb(_rb(x - _rb(mean)) * (1.0 / sd))


def _sigmoid(x):
    return 1.0 / (1.0 + jnp.exp(-x))


def _silu(x):
    return x * _sigmoid(x)


def _kernel(x_hbm, mem0_hbm, wq_hbm, wk_hbm, wv_hbm, wo_hbm, wr_hbm, wg_hbm, wu_hbm, wd_hbm,
            out_hbm,
            x_s, xe_s, xen_s, raw_s, w_s, wo_s, wg_s, wu_s, wd_s, act_s, r_s, out_s, mem0_s, wr_s,
            sem, sem_out):
    n_seg, seg, D = x_hbm.shape
    S = n_seg * seg
    H, E = wq_hbm.shape[1], wq_hbm.shape[2]
    M = mem0_hbm.shape[0]
    L = seg + M
    n_col = D // LANES
    n_pair = 3 * H // 2
    n_early = n_seg * EARLY_ROWS
    seg_blk = n_seg // N_BLK
    rows_blk = seg_blk * seg
    pair_blk = (n_pair - FIRST_PAIRS - LAST_PAIRS) // N_BLK
    assert FIRST_PAIRS + N_BLK * pair_blk + LAST_PAIRS == n_pair
    assert rows_blk // SUBLANES <= LANES

    XN, GATE, EARLY = 0, n_col * S, 2 * n_col * S

    def act_load(base, r, n):
        return jnp.concatenate([act_s[pl.ds(base + c * S + r, n), :] for c in range(n_col)],
                               axis=1)

    def act_store(base, r, val, stride=S):
        for c in range(val.shape[1] // LANES):
            act_s[pl.ds(base + c * stride + r, val.shape[0]), :] = val[:, c * LANES:(c + 1) * LANES]

    SEM_EARLY, SEM_FIRST = 0, EARLY_PARTS
    SEM_BLK = SEM_FIRST + FIRST_PAIRS
    SEM_X = SEM_BLK + N_BLK
    SEM_SMALL, SEM_LAST, SEM_FFN, SEM_WO = (SEM_X + N_BLK + i for i in range(4))

    seg_part = n_seg // EARLY_PARTS
    early_copies = [
        pltpu.make_async_copy(x_hbm.at[pl.ds(i * seg_part, seg_part), pl.ds(0, EARLY_ROWS), :],
                              xe_s.at[pl.ds(i * seg_part, seg_part)], sem.at[SEM_EARLY + i])
        for i in range(EARLY_PARTS)]
    small_copies = [pltpu.make_async_copy(src, dst, sem.at[SEM_SMALL])
                    for src, dst in ((wr_hbm, wr_s), (mem0_hbm, mem0_s))]
    ffn_copies = [pltpu.make_async_copy(src, dst, sem.at[SEM_FFN])
                  for src, dst in ((wg_hbm, wg_s), (wu_hbm, wu_s), (wd_hbm, wd_s))]
    wo_copies = [pltpu.make_async_copy(wo_hbm.at[:, pl.ds(n * LANES, LANES)], wo_s.at[n],
                                       sem.at[SEM_WO]) for n in range(n_col)]

    def x_copy(i):
        blk = pl.ds(i * seg_blk, seg_blk)
        return pltpu.make_async_copy(x_hbm.at[blk], x_s.at[blk], sem.at[SEM_X + i])

    def pairs_start(p0, n, sem_id):
        for p in range(p0, p0 + n):
            m, c = divmod(p, H // 2)
            src = (wq_hbm, wk_hbm, wv_hbm)[m].bitcast(U32).at[:, c, :]
            pltpu.make_async_copy(src, raw_s.at[p], sem.at[sem_id]).start()

    def pairs_wait(p0, n, sem_id):
        dst = raw_s.at[pl.ds(p0, n)]
        pltpu.make_async_copy(dst, dst, sem.at[sem_id]).wait()

    for cp in early_copies:
        cp.start()
    for p in range(FIRST_PAIRS):
        pairs_start(p, 1, SEM_FIRST + p)
    for cp in small_copies:
        cp.start()
    for i in range(N_BLK):
        pairs_start(FIRST_PAIRS + i * pair_blk, pair_blk, SEM_BLK + i)
        x_copy(i).start()
    pairs_start(n_pair - LAST_PAIRS, LAST_PAIRS, SEM_LAST)
    for cp in ffn_copies + wo_copies:
        cp.start()

    def project_early(p0, n, side_work):
        n_piece = n * (n_early // EARLY_M)
        piece = done = 0
        for j in range(n):
            p = p0 + j
            even = raw_s[p, pl.ds(0, D // 2, stride=2), :]
            odd = raw_s[p, pl.ds(1, D // 2, stride=2), :]
            lo = (even & np.uint32(0xFFFF)) | (odd << 16)
            hi = (even >> 16) | (odd & np.uint32(0xFFFF0000))
            w_s[2 * p] = lo
            w_s[2 * p + 1] = hi
            w = jnp.concatenate([pltpu.bitcast(lo, BF16), pltpu.bitcast(hi, BF16)], axis=1)
            for r in range(0, n_early, EARLY_M):
                res = _dot(xen_s[r:r + EARLY_M, :], w)
                act_store(EARLY, _aligned(2 * p * n_early + r, EARLY_M), res, n_early)
                piece += 1
                while done < min(len(side_work), -(-piece * len(side_work) // (n_piece - 2))):
                    side_work[done]()
                    done += 1

    lane8 = lax.broadcasted_iota(I32, (SUBLANES, LANES), 1)

    def norm_work(blk, wr):
        scores = [jnp.zeros((SUBLANES, LANES), F32)]
        n = rows_blk // SUBLANES

        def piece(i):
            sg, off = divmod(i * SUBLANES, seg)
            xn = _layernorm(x_s[blk * seg_blk + sg, off:off + SUBLANES, :].astype(F32))
            r0 = _aligned(blk * rows_blk + i * SUBLANES, SUBLANES)
            act_store(XN, r0, xn)
            act_store(GATE, r0, _silu(xn + xn * 0.0))
            scores[0] = jnp.where(lane8 == i, jnp.sum(xn * wr, axis=-1, keepdims=True), scores[0])
            if i == n - 1:
                r_s[blk] = scores[0]

        return [functools.partial(piece, i) for i in range(n)]

    def routed_ffn_work():
        st = {}

        def select():
            idx_bits = (S - 1).bit_length()
            int_min = np.int32(-2 ** 31)
            r_all = _rb(r_s[...].reshape(N_BLK * SUBLANES, LANES))
            r_all = jnp.where(r_all == 0.0, 0.0, r_all)
            bits = lax.bitcast_convert_type(r_all, I32) >> 16
            code = jnp.where(bits < 0, bits ^ 0x7FFF, bits)
            code = jnp.where(r_all != r_all, -32768, code)
            row = lax.broadcasted_iota(I32, r_all.shape, 0)
            col = lax.broadcasted_iota(I32, r_all.shape, 1)
            tok = (row >> 3) * rows_blk + col * SUBLANES + (row & 7)
            keys = jnp.where(col < rows_blk // SUBLANES, (code << idx_bits) | (S - 1 - tok),
                             int_min)
            row_c = lax.broadcasted_iota(I32, (TOP_C, LANES), 0)
            best_keys = jnp.zeros((TOP_C, LANES), I32)
            for c in range(TOP_C):
                best = jnp.max(jnp.max(keys, axis=0, keepdims=True), axis=1, keepdims=True)
                best_keys = jnp.where(row_c == c, best, best_keys)
                keys = jnp.where(keys == best, int_min, keys)
            best_code = best_keys >> idx_bits
            st["score"] = lax.bitcast_convert_type(
                jnp.where(best_code < 0, best_code ^ 0x7FFF, best_code) << 16, F32)
            best_tok = S - 1 - (best_keys & (2 ** idx_bits - 1))
            st["idx"] = [jnp.max(jnp.where(row_c == c, best_tok, 0)) for c in range(TOP_C)]

        def gather():
            st["x"] = jnp.concatenate([act_load(XN, t, 1) for t in st["idx"]], axis=0)
            st["h"] = []

        def hidden(f0, f1):
            gate = _rb(_dot(st["x"], wg_s[f0:f1, :], _NT))
            up = _rb(_dot(st["x"], wu_s[f0:f1, :], _NT))
            st["h"].append(_silu(gate) * up)

        def down():
            st["y"] = _dot(jnp.concatenate(st["h"], axis=1), wd_s[...])

        def scatter():
            y = _rb(st["y"]) * _sigmoid(st["score"][:, :1])
            gate = _silu(st["x"] + (st["x"] * 0.0 + y))
            for c, t in enumerate(st["idx"]):
                act_store(GATE, t, gate[c:c + 1])

        def pause():
            pass

        n_f = wg_s.shape[0]
        return ([select] + [pause] * 8 + [gather]
                + [functools.partial(hidden, f, min(f + FFN_COLS, n_f))
                   for f in range(0, n_f, FFN_COLS)]
                + [pause, down, pause, scatter])

    for i, cp in enumerate(early_copies):
        cp.wait()
        n = seg_part * EARLY_ROWS
        xe = xe_s[i * seg_part:(i + 1) * seg_part].astype(F32).reshape(n, D)
        xen_s[i * n:(i + 1) * n, :] = _layernorm(xe).astype(BF16)

    def first_pair(p, carry):
        pairs_wait(p, 1, SEM_FIRST + p)
        project_early(p, 1, [])
        return carry

    lax.fori_loop(0, FIRST_PAIRS, first_pair, 0)

    for cp in small_copies:
        cp.wait()
    wr = wr_s[...].astype(F32).reshape(1, D)

    def middle_block(i, carry):
        p0 = FIRST_PAIRS + i * pair_blk
        pairs_wait(p0, pair_blk, SEM_BLK + i)
        x_copy(i).wait()
        project_early(p0, pair_blk, norm_work(i, wr))
        return carry

    lax.fori_loop(0, N_BLK, middle_block, 0)

    pairs_wait(n_pair - LAST_PAIRS, LAST_PAIRS, SEM_LAST)
    for cp in ffn_copies:
        cp.wait()
    project_early(n_pair - LAST_PAIRS, LAST_PAIRS, routed_ffn_work())
    for cp in wo_copies:
        cp.wait()

    scale = E ** -0.5
    per_tile = LANES // L
    groups = [list(range(h, min(h + per_tile, H))) for h in range(0, H, per_tile)]
    n_g = len(groups)
    lane = lax.broadcasted_iota(I32, (L, LANES), 1)
    key_j = lax.broadcasted_iota(I32, (L, LANES), 0)
    qry_t = lane
    for i in range(1, per_tile):
        qry_t = jnp.where(lane >= i * L, lane - i * L, qry_t)
    allowed = (qry_t >= seg) | (key_j >= seg) | (key_j <= qry_t)
    wo_words = wo_s.bitcast(U32)

    def probabilities(q, k):
        n = len(q)
        qs = jnp.concatenate(q + [jnp.zeros((LANES - n * L, E), F32)], axis=0).astype(BF16)
        st = _dot(jnp.concatenate(k, axis=0), qs, _NT)
        merged = st[:L]
        for i in range(1, n):
            merged = jnp.where(lane >= i * L, st[i * L:(i + 1) * L], merged)
        sc = jnp.where(allowed, merged * scale, -1e9)
        e = jnp.exp(sc - jnp.max(sc, axis=0, keepdims=True))
        return e / jnp.sum(e, axis=0, keepdims=True)

    def mix(pt, v):
        p = jnp.concatenate([pt, jnp.zeros((LANES - L, LANES), F32)], axis=0).T
        outs = []
        for i, vh in enumerate(v):
            vp = jnp.concatenate([vh, jnp.zeros((LANES - L, E), F32)], axis=0).astype(BF16)
            o = _dot(p[i * L:(i + 1) * L], vp)
            outs.append(jnp.concatenate([o[seg:], o[:seg]], axis=0))
        return outs

    def out_proj(n, outs, h0):
        rows = slice(h0 * E // 2, (h0 + len(outs)) * E // 2)
        return _dot(jnp.concatenate(outs, axis=1), pltpu.bitcast(wo_words[n, rows, :], BF16))

    def step(s, mem):
        r0 = pl.multiple_of(s * seg, seg)
        e0 = pl.multiple_of(s * EARLY_ROWS, EARLY_ROWS)
        h = jnp.concatenate([act_load(XN + EARLY_ROWS, r0, seg - EARLY_ROWS), mem],
                            axis=0).astype(BF16)

        def project(m, heads, k0=0, k1=D):
            w = jnp.concatenate(
                [pltpu.bitcast(w_s[m * H + hd, k0 // 2:k1 // 2, :], BF16) for hd in heads], axis=1)
            return _dot(h[:, k0:k1], w)

        def with_early(m, heads, res):
            return [jnp.concatenate(
                [act_s[pl.ds(EARLY + (m * H + hd) * n_early + e0, EARLY_ROWS), :],
                 res[:, j * E:(j + 1) * E]], axis=0) for j, hd in enumerate(heads)]

        k_split = D - LANES
        head_start = [project(m, groups[0], 0, k_split) for m in range(2)]
        q, k, v, probs, o = {}, {}, {}, {}, {}
        for t in range(2 * n_g):
            if t < n_g:
                for m, dst in enumerate((q, k)):
                    if t == 0:
                        res = project(m, groups[t], k_split, D) + head_start[m]
                    else:
                        res = project(m, groups[t])
                    dst[t] = with_early(m, groups[t], res)
            else:
                v[t - n_g] = with_early(2, groups[t - n_g], project(2, groups[t - n_g]))
            g = t - LAG_SCORES
            if 0 <= g < n_g:
                probs[g] = probabilities(q[g], k[g])
            g = t - n_g - LAG_MIX
            if 0 <= g < n_g:
                o[g] = mix(probs[g], v[g])

        n_done = n_g - LAG_MIX
        ready = [oh for g in range(n_done) for oh in o[g]]
        cuts = [len(ready) * i // LAG_MIX for i in range(LAG_MIX + 1)]
        col0, late = None, []
        for i in range(LAG_MIX):
            part = out_proj(0, ready[cuts[i]:cuts[i + 1]], cuts[i])
            col0 = part if col0 is None else part + col0
            late += mix(probs[n_done + i], v[n_done + i])
        col1 = out_proj(1, ready + late, 0)
        col0 = out_proj(0, late, len(ready)) + col0
        res = jnp.concatenate(
            [col0, col1] + [out_proj(n, ready + late, 0) for n in range(2, n_col)], axis=1)

        out_s[s] = (x_s[s].astype(F32) + res[M:] * act_load(GATE, r0, seg)).astype(BF16)
        pltpu.make_async_copy(out_s.at[s], out_hbm.at[s], sem_out).start()
        return res[:M]

    lax.fori_loop(0, n_seg, step, mem0_s[...].astype(F32), unroll=UNROLL)
    pltpu.make_async_copy(out_s, out_s, sem_out).wait()


@functools.partial(jax.jit, static_argnames=("A_seg_len",))
def pallas_recurrent_scan__memory_aug_recurrent_mem_tr__moe_arch_mod__prompt_kernel(
    A_x: jax.Array,
    A_mem0: jax.Array,
    A_Wq: jax.Array,
    A_Wk: jax.Array,
    A_Wv: jax.Array,
    A_Wo: jax.Array,
    A_seg_len: int,
    B_x: jax.Array,
    B_w_r: jax.Array,
    B_w_gate: jax.Array,
    B_w_up: jax.Array,
    B_w_down: jax.Array,
):
    del B_x
    B, S, D = A_x.shape
    _, H, E = A_Wq.shape
    M = A_mem0.shape[1]
    F = B_w_gate.shape[1]
    seg = int(A_seg_len)
    n_seg = S // seg
    n_col = D // LANES
    assert B == 1 and E == LANES and D % LANES == 0 and S == n_seg * seg

    hbm = pl.BlockSpec(memory_space=pltpu.HBM)
    out = pl.pallas_call(
        _kernel,
        out_shape=jax.ShapeDtypeStruct((n_seg, seg, D), A_x.dtype),
        in_specs=[hbm] * 10,
        out_specs=hbm,
        scratch_shapes=[
            pltpu.VMEM((n_seg, seg, D), BF16),
            pltpu.VMEM((n_seg, EARLY_ROWS, D), BF16),
            pltpu.VMEM((n_seg * EARLY_ROWS, D), BF16),
            pltpu.VMEM((3 * H // 2, D, E), U32),
            pltpu.VMEM((3 * H, D // 2, E), U32),
            pltpu.VMEM((n_col, H * E, LANES), BF16),
            pltpu.VMEM((F, D), BF16),
            pltpu.VMEM((F, D), BF16),
            pltpu.VMEM((F, D), BF16),
            pltpu.VMEM((2 * n_col * S + 3 * H * n_seg * EARLY_ROWS, LANES), F32),
            pltpu.VMEM((N_BLK, SUBLANES, LANES), F32),
            pltpu.VMEM((n_seg, seg, D), BF16),
            pltpu.VMEM((M, D), BF16),
            pltpu.VMEM((D,), BF16),
            pltpu.SemaphoreType.DMA((EARLY_PARTS + FIRST_PAIRS + 2 * N_BLK + 4,)),
            pltpu.SemaphoreType.DMA(()),
        ],
        compiler_params=pltpu.CompilerParams(vmem_limit_bytes=110 * 1024 * 1024),
    )(A_x.reshape(n_seg, seg, D), A_mem0.reshape(M, D), A_Wq, A_Wk, A_Wv, A_Wo.reshape(H * E, D),
      B_w_r, B_w_gate.T, B_w_up.T, B_w_down)
    return out.reshape(B, S, D)
```
